```python
import jax
import jax.numpy as jnp

def _softmax(x, axis=-1):
    return jax.nn.softmax(x, axis=axis)
def _gelu(x):
    return jax.nn.gelu(x, approximate=True)
def _silu(x):
    return jax.nn.silu(x)
def _sigmoid(x):
    return jax.nn.sigmoid(x)
def _layernorm(x, axis=-1, eps=1e-5):
    m = jnp.mean(x, axis=axis, keepdims=True)
    v = jnp.var(x, axis=axis, keepdims=True)
    return (x - m) / jnp.sqrt(v + eps)
def _scatter_add(tgt, idx, src, axis=0):
    return tgt.at[idx].add(src)
def _segment_sum(src, seg, n):
    return jax.ops.segment_sum(src, seg, n)
class _Rng:
    def __init__(self, key):
        self._k = key
    def _next(self):
        self._k, sub = jax.random.split(self._k)
        return sub
    def normal(self, shape):
        return jax.random.normal(self._next(), shape, dtype=jnp.bfloat16)
    def randint(self, lo, hi, shape):
        return jax.random.randint(self._next(), shape, lo, hi, dtype=jnp.int32)
    def uniform(self, shape, lo=0.0, hi=1.0):
        return jax.random.uniform(self._next(), shape, jnp.bfloat16, lo, hi)
    def permutation(self, n):
        return jax.random.permutation(self._next(), n)


kernel_name = 'gated_mix__ssm_conv_h3__compressed_kv_cla__prompt'

def setup_inputs():
    _rng = _Rng(jax.random.key(int.from_bytes(__import__("os").urandom(4), "little")))
    _w = (lambda a: (lambda t: t.astype(jnp.bfloat16) if jnp.issubdtype(t.dtype, jnp.floating) else t)(jnp.asarray(a)))
    def _A_setup():
        B, S, D = 1, 2048, 1024
        ks = 4
        return {
            "q": _w((lambda *s: _rng.normal(s) * 0.05)(B, S, D)),
            "k": _w((lambda *s: _rng.normal(s) * 0.05)(B, S, D)),
            "v": _w((lambda *s: _rng.normal(s) * 0.05)(B, S, D)),
            "shift_k": _w((lambda *s: _rng.normal(s) * 0.05)(D, ks) * 0.5),
            "ssm_k": _w((lambda *s: _rng.normal(s) * 0.05)(D, S) * (1.0 / S ** 0.5)),
            "ssm_D": _w((lambda *s: _rng.normal(s) * 0.05)(D)),
        }
    _A_in = _A_setup()

    def _B_setup():
        B, H, Sq, Sk, D, M = 1, 32, 2048, 2048, 128, 1024
        Dc = 4 * D
        return {
            "x": _w((lambda *s: _rng.normal(s) * 0.05)(B, Sq, M)),
            "c_kv": _w((lambda *s: _rng.normal(s) * 0.05)(B, Sk, Dc)),
            "w_q": _w((lambda *s: _rng.normal(s) * 0.05)(M, H, D) * (M ** -0.5)),
            "w_uk": _w((lambda *s: _rng.normal(s) * 0.05)(Dc, H, D) * (Dc ** -0.5)),
            "w_uv": _w((lambda *s: _rng.normal(s) * 0.05)(Dc, H, D) * (Dc ** -0.5)),
            "w_o": _w((lambda *s: _rng.normal(s) * 0.05)(H, D, M) * ((H * D) ** -0.5)),
        }
    _B_in = _B_setup()

    return {
        "A_q": _A_in["q"],
        "A_k": _A_in["k"],
        "A_v": _A_in["v"],
        "A_shift_k": _A_in["shift_k"],
        "A_ssm_k": _A_in["ssm_k"],
        "A_ssm_D": _A_in["ssm_D"],
        "B_x": _B_in["x"],
        "B_c_kv": _B_in["c_kv"],
        "B_w_q": _B_in["w_q"],
        "B_w_uk": _B_in["w_uk"],
        "B_w_uv": _B_in["w_uv"],
        "B_w_o": _B_in["w_o"],
        "gate_w": _w((lambda *s: _rng.normal(s) * 0.05)(1024)),
    }

def reference(A_q, A_k, A_v, A_shift_k, A_ssm_k, A_ssm_D, B_x, B_c_kv, B_w_q, B_w_uk, B_w_uv, B_w_o, gate_w):
    def _A_ref(q, k, v, shift_k, ssm_k, ssm_D):
        B, S, D = q.shape
        ks = shift_k.shape[-1]
        k_pad = jnp.pad(k, ((0, 0), (ks - 1, 0), (0, 0)))
        k_shift = jnp.zeros_like(k)
        for t in range(ks):
            k_shift = k_shift + k_pad[:, t:t + S, :] * shift_k[:, ks - 1 - t][None, None, :]
        kv = k_shift * v
        L = 2 * S
        kv_pad = jnp.pad(kv, ((0, 0), (0, S), (0, 0)))
        kf_pad = jnp.pad(ssm_k, ((0, 0), (0, S)))
        kv_f = (lambda x, axes=(-2,-1): jnp.fft.rfft2(x.astype(jnp.float32), axes=axes))(kv_pad[:, None, :, :], axes=(1, 2))
        kf_f = (lambda x, axes=(-2,-1): jnp.fft.rfft2(x.astype(jnp.float32), axes=axes))(kf_pad[:, None, :], axes=(1, 2))
        kf_f = (lambda x, *d: x.transpose(*d))(kf_f, 1, 2, 0)
        y_f = kv_f * kf_f[None, :, :, :]
        y = (lambda x, s, axes=(-2,-1): jnp.fft.irfft2(x, s=s, axes=axes).astype(jnp.bfloat16))(y_f, (1, L), axes=(1, 2))[:, 0, :S, :]
        y = y + kv * ssm_D[None, None, :]
        return q * y

    def _B_ref(x, c_kv, w_q, w_uk, w_uv, w_o):
        B, Sq, M = x.shape[0], x.shape[1], x.shape[2]
        Sk = c_kv.shape[1]
        H, D = w_q.shape[1], w_q.shape[2]
        q = jnp.einsum("bqm,mhd->bhqd", x, w_q)
        k = jnp.einsum("bkc,chd->bhkd", c_kv, w_uk)
        v = jnp.einsum("bkc,chd->bhkd", c_kv, w_uv)
        scores = jnp.einsum("bhqd,bhkd->bhqk", q, k) * (D ** -0.5)
        off = Sk - Sq
        qi = jnp.arange(Sq)[:, None]
        kj = jnp.arange(Sk)[None, :]
        cmask = kj <= (qi + off)
        scores = jnp.where(cmask[None, None], scores, -1e9)
        p = _softmax(scores, axis=-1)
        ctx = jnp.einsum("bhqk,bhkd->bhqd", p, v)
        return jnp.einsum("bhqd,hdm->bqm", ctx, w_o)

    x = A_q
    g = _sigmoid((x * gate_w).sum(-1, keepdims=True))
    a = _A_ref(x, A_k, A_v, A_shift_k, A_ssm_k, A_ssm_D)
    b = _B_ref(x, B_c_kv, B_w_q, B_w_uk, B_w_uv, B_w_o)
    return g * a + (1 - g) * b
```

```python
import numpy as np

import jax
import jax.numpy as jnp
from jax import lax
import jax.experimental.pallas as pl
import jax.experimental.pallas.tpu as pltpu

S = 2048
DM = 1024
H = 32
HD = 128
DC = 512
CB = 128
NB = S // CB
CG = 128
NG = DM // CG
BQ = 256

LOG2E = 1.4426950408889634
NT = (((1,), (1,)), ((), ()))


def _dft_matrices():
    n = 2 * CB
    f = np.concatenate([np.arange(0, CB, 2), np.arange(1, CB, 2)]).astype(np.float64)
    j = np.arange(CB, dtype=np.float64)
    ang = 2.0 * np.pi * np.outer(f + 0.5, j) / n
    fwd = np.concatenate([np.cos(ang), -np.sin(ang)], axis=0)
    inv = np.concatenate([np.cos(ang).T, -np.sin(ang).T], axis=1)
    inv = inv * (2.0 / n)
    return fwd.astype(np.float32), inv.astype(np.float32)


_FWD_NP, _INV_NP = _dft_matrices()


def _head_weight(w32, h):
    sh = (16 - 16 * (h & 1)).astype(jnp.uint32)
    w = (w32 << sh) & jnp.uint32(0xFFFF0000)
    return pltpu.bitcast(w, jnp.float32).astype(jnp.bfloat16)


def _kernel(x_ref, c_ref, wq_ref, wuk_ref, wuv_ref, gw_ref, fwd_ref, inv_ref,
            xq_ref, ak_ref, av_ref, sk_ref, hk_ref, sd_ref, wo_ref,
            o_ref,
            q_s, k_s, v_s, ctx_s, g_s, kp_s, xf_s, hf_s, z_s, b_s, kv_s,
            wq_b, wuk_b, wuv_b, wsem):
    step = pl.program_id(0)

    def w_copies(pair):
        slot = pair & 1
        return [
            pltpu.make_async_copy(src.bitcast(jnp.uint32).at[:, pair, :], dst.at[slot], wsem.at[n, slot])
            for n, (src, dst) in enumerate(((wq_ref, wq_b), (wuk_ref, wuk_b), (wuv_ref, wuv_b)))
        ]

    @pl.when(step == 0)
    def _first_weights():
        for cp in w_copies(0):
            cp.start()

    @pl.when((step < H) & ((step & 1) == 0))
    def _next_weights():
        pair = step >> 1

        @pl.when(pair + 1 < H // 2)
        def _():
            for cp in w_copies(pair + 1):
                cp.start()

        for cp in w_copies(pair):
            cp.wait()

    @pl.when(step < H)
    def _attention():
        h = step
        rows = S // H
        r0 = pl.multiple_of(h * rows, rows)
        xg = x_ref[pl.ds(r0, rows), :].astype(jnp.float32) * gw_ref[...].astype(jnp.float32)
        gl = jnp.sum(xg, axis=-1, keepdims=True)
        g_s[pl.ds(r0, rows), :] = jnp.broadcast_to(jax.nn.sigmoid(gl), (rows, CG))

        slot = (h >> 1) & 1
        wq = _head_weight(wq_b[slot], h)
        wkv = jnp.concatenate([_head_weight(wuk_b[slot], h), _head_weight(wuv_b[slot], h)], axis=1)
        kv = jnp.dot(c_ref[...], wkv, preferred_element_type=jnp.float32)
        k_s[...] = kv[:, :HD].astype(jnp.bfloat16)
        v_s[...] = kv[:, HD:].astype(jnp.bfloat16)
        q = jnp.dot(x_ref[...], wq, preferred_element_type=jnp.float32)
        q_s[...] = (q * (HD ** -0.5 * LOG2E)).astype(jnp.bfloat16)

        row = lax.broadcasted_iota(jnp.int32, (BQ, BQ), 0)
        col = lax.broadcasted_iota(jnp.int32, (BQ, BQ), 1)
        for i in range(S // BQ):
            kvl = (i + 1) * BQ
            s = lax.dot_general(q_s[i * BQ:(i + 1) * BQ, :], k_s[:kvl, :], NT,
                                preferred_element_type=jnp.float32)
            sd = jnp.where(col <= row, s[:, kvl - BQ:], -1e9 * LOG2E)
            s = sd if i == 0 else jnp.concatenate([s[:, :kvl - BQ], sd], axis=1)
            m = jnp.max(s, axis=-1, keepdims=True)
            p = jnp.exp2(s - m)
            l = jnp.sum(p, axis=-1, keepdims=True)
            o = jnp.dot(p.astype(jnp.bfloat16), v_s[:kvl, :], preferred_element_type=jnp.float32)
            ctx_s[h, i * BQ:(i + 1) * BQ, :] = (o / l).astype(jnp.bfloat16)

    @pl.when(step >= H)
    def _mix():
        def out_proj(j):
            r = slice(j * CB, (j + 1) * CB)
            lhs = jnp.concatenate([ctx_s[hh, r, :] for hh in range(H)], axis=1)
            b = jnp.dot(lhs, wo_ref[...], preferred_element_type=jnp.float32)
            b_s[r, :] = (1.0 - g_s[r, :]) * b

        kp_s[0:8, :] = jnp.zeros((8, CG), jnp.float32)
        kp_s[8:, :] = ak_ref[...].astype(jnp.float32)
        sk = sk_ref[...].astype(jnp.float32)
        fwd = fwd_ref[...]
        out_proj(0)
        for i in range(NB):
            acc = kp_s[8 + i * CB:8 + (i + 1) * CB, :] * sk[0:1, :]
            for t in range(1, 4):
                acc = acc + kp_s[8 - t + i * CB:8 - t + (i + 1) * CB, :] * sk[t:t + 1, :]
            kvb = (acc * av_ref[i * CB:(i + 1) * CB, :].astype(jnp.float32)).astype(jnp.bfloat16)
            kv_s[i * CB:(i + 1) * CB, :] = kvb
            xf_s[i] = jnp.dot(fwd, kvb, preferred_element_type=jnp.float32)
        out_proj(1)
        hq = CB // 2
        prev = None
        for m in range(NB):
            hf = lax.dot_general(fwd, hk_ref[:, m * CB:(m + 1) * CB], NT,
                                 preferred_element_type=jnp.float32)
            if prev is None:
                hf_s[m] = hf
            else:
                hf_s[m, 0:hq, :] = hf[0:hq] - prev[2 * hq:3 * hq]
                hf_s[m, hq:2 * hq, :] = hf[hq:2 * hq] + prev[3 * hq:4 * hq]
                hf_s[m, 2 * hq:3 * hq, :] = hf[2 * hq:3 * hq] + prev[0:hq]
                hf_s[m, 3 * hq:4 * hq, :] = hf[3 * hq:4 * hq] - prev[hq:2 * hq]
            prev = hf
        TI = 4
        nchunk = CB // 16
        for fc in range(nchunk):
            for half in range(2):
                f0 = fc * 16 + half * 8
                re = slice(f0, f0 + 8)
                im = slice(CB + f0, CB + f0 + 8)
                for i0 in range(0, NB, TI):
                    ar = [None] * TI
                    ai = [None] * TI
                    for m in range(i0 + TI):
                        gr = hf_s[m, re, :]
                        gi = hf_s[m, im, :]
                        for u in range(TI):
                            d = i0 + u - m
                            if d < 0:
                                continue
                            xr = xf_s[d, re, :]
                            xi = xf_s[d, im, :]
                            pr = gr * xr - gi * xi
                            pi = gr * xi + gi * xr
                            ar[u] = pr if ar[u] is None else ar[u] + pr
                            ai[u] = pi if ai[u] is None else ai[u] + pi
                    for u in range(TI):
                        z_s[i0 + u, re, :] = ar[u]
                        z_s[i0 + u, im, :] = ai[u]
            if fc < nchunk - 1:
                out_proj(2 + 2 * fc)
                out_proj(3 + 2 * fc)
        inv = inv_ref[...]
        sd = sd_ref[...].astype(jnp.float32)
        for i in range(NB):
            r = slice(i * CB, (i + 1) * CB)
            y = jnp.dot(inv, z_s[i].astype(jnp.bfloat16), preferred_element_type=jnp.float32)
            a = xq_ref[r, :].astype(jnp.float32) * (y + kv_s[r, :].astype(jnp.float32) * sd)
            o_ref[r, :] = (g_s[r, :] * a + b_s[r, :]).astype(o_ref.dtype)


@jax.jit
def pallas_gated_mix__ssm_conv_h3__compressed_kv_cla__prompt_kernel(
    A_q: jax.Array,
    A_k: jax.Array,
    A_v: jax.Array,
    A_shift_k: jax.Array,
    A_ssm_k: jax.Array,
    A_ssm_D: jax.Array,
    B_x: jax.Array,
    B_c_kv: jax.Array,
    B_w_q: jax.Array,
    B_w_uk: jax.Array,
    B_w_uv: jax.Array,
    B_w_o: jax.Array,
    gate_w: jax.Array,
):
    del B_x
    x = A_q.reshape(S, DM)
    fwd = jnp.asarray(_FWD_NP, dtype=jnp.bfloat16)
    inv = jnp.asarray(_INV_NP, dtype=jnp.bfloat16)

    one = pl.Buffered(1)

    def whole(shape):
        return pl.BlockSpec(shape, lambda s: (0,) * len(shape), pipeline_mode=one)

    def grp(s):
        return jnp.maximum(s - H, 0)

    col = lambda rows: pl.BlockSpec((rows, CG), lambda s: (0, grp(s)))

    out = pl.pallas_call(
        _kernel,
        grid=(H + NG,),
        in_specs=[
            whole((S, DM)),
            whole((S, DC)),
            pl.BlockSpec(memory_space=pl.ANY),
            pl.BlockSpec(memory_space=pl.ANY),
            pl.BlockSpec(memory_space=pl.ANY),
            whole((1, DM)),
            whole((2 * CB, CB)),
            whole((CB, 2 * CB)),
            col(S),
            col(S),
            col(S),
            col(4),
            pl.BlockSpec((CG, S), lambda s: (grp(s), 0)),
            col(1),
            col(H * HD),
        ],
        out_specs=col(S),
        out_shape=jax.ShapeDtypeStruct((S, DM), jnp.bfloat16),
        scratch_shapes=[
            pltpu.VMEM((S, HD), jnp.bfloat16),
            pltpu.VMEM((S, HD), jnp.bfloat16),
            pltpu.VMEM((S, HD), jnp.bfloat16),
            pltpu.VMEM((H, S, HD), jnp.bfloat16),
            pltpu.VMEM((S, CG), jnp.float32),
            pltpu.VMEM((S + 8, CG), jnp.float32),
            pltpu.VMEM((NB, 2 * CB, CG), jnp.float32),
            pltpu.VMEM((NB, 2 * CB, CG), jnp.float32),
            pltpu.VMEM((NB, 2 * CB, CG), jnp.float32),
            pltpu.VMEM((S, CG), jnp.float32),
            pltpu.VMEM((S, CG), jnp.bfloat16),
            pltpu.VMEM((2, DM, HD), jnp.uint32),
            pltpu.VMEM((2, DC, HD), jnp.uint32),
            pltpu.VMEM((2, DC, HD), jnp.uint32),
            pltpu.SemaphoreType.DMA((3, 2)),
        ],
        compiler_params=pltpu.CompilerParams(
            dimension_semantics=("arbitrary",),
            vmem_limit_bytes=110 * 1024 * 1024,
        ),
    )(
        x,
        B_c_kv.reshape(S, DC),
        B_w_q,
        B_w_uk,
        B_w_uv,
        gate_w.reshape(1, DM),
        fwd,
        inv,
        x,
        A_k.reshape(S, DM),
        A_v.reshape(S, DM),
        A_shift_k.T,
        A_ssm_k,
        A_ssm_D.reshape(1, DM),
        B_w_o.reshape(H * HD, DM),
    )
    return out.reshape(1, S, DM)
```

```python
import numpy as np

import jax
import jax.numpy as jnp
from jax import lax
import jax.experimental.pallas as pl
import jax.experimental.pallas.tpu as pltpu

S = 2048
DM = 1024
H = 32
HD = 128
DC = 512
CB = 128
NB = S // CB
CG = 128
NG = DM // CG
BQ = 256
NQ = S // BQ

LOG2E = 1.4426950408889634
NT = (((1,), (1,)), ((), ()))


def _dft_matrices():
    n = 2 * CB
    f = np.concatenate([np.arange(0, CB, 2), np.arange(1, CB, 2)]).astype(np.float64)
    j = np.arange(CB, dtype=np.float64)
    ang = 2.0 * np.pi * np.outer(f + 0.5, j) / n
    fwd = np.concatenate([np.cos(ang), -np.sin(ang)], axis=0)
    inv = np.concatenate([np.cos(ang).T, -np.sin(ang).T], axis=1)
    inv = inv * (2.0 / n)
    return fwd.astype(np.float32), inv.astype(np.float32)


_FWD_NP, _INV_NP = _dft_matrices()


def _head_weight(w32, h):
    sh = (16 - 16 * (h & 1)).astype(jnp.uint32)
    w = (w32 << sh) & jnp.uint32(0xFFFF0000)
    return pltpu.bitcast(w, jnp.float32).astype(jnp.bfloat16)


def _kernel(x_ref, c_ref, wq_ref, wuk_ref, wuv_ref, gw_ref, fwd_ref, inv_ref,
            xq_ref, ak_ref, av_ref, sk_ref, hk_ref, sd_ref, wo_ref,
            o_ref,
            q_s, k_s, v_s, ctx_s, g_s, kp_s, xf_s, hf_s, z_s, b_s, kv_s,
            wq_b, wuk_b, wuv_b, wq_s, wkv_s, wsem):
    step = pl.program_id(0)

    def w_copies(pair):
        slot = pair & 1
        return [
            pltpu.make_async_copy(src.bitcast(jnp.uint32).at[:, pair, :], dst.at[slot], wsem.at[n, slot])
            for n, (src, dst) in enumerate(((wq_ref, wq_b), (wuk_ref, wuk_b), (wuv_ref, wuv_b)))
        ]

    def unpack_q(h):
        wq_s[...] = _head_weight(wq_b[(h >> 1) & 1], h)

    def unpack_kv(h):
        slot = (h >> 1) & 1
        wkv_s[:, :HD] = _head_weight(wuk_b[slot], h)
        wkv_s[:, HD:] = _head_weight(wuv_b[slot], h)

    def q_proj(i):
        r = slice(i * BQ, (i + 1) * BQ)
        q = jnp.dot(x_ref[r, :], wq_s[...], preferred_element_type=jnp.float32)
        q_s[r, :] = (q * (HD ** -0.5 * LOG2E)).astype(jnp.bfloat16)

    def kv_proj(i):
        r = slice(i * BQ, (i + 1) * BQ)
        kv = jnp.dot(c_ref[r, :], wkv_s[...], preferred_element_type=jnp.float32)
        k_s[r, :] = kv[:, :HD].astype(jnp.bfloat16)
        v_s[r, :] = kv[:, HD:].astype(jnp.bfloat16)

    @pl.when(step == 0)
    def _first_head():
        for cp in w_copies(0) + w_copies(1):
            cp.start()
        for cp in w_copies(0):
            cp.wait()
        unpack_kv(step)
        unpack_q(step)
        for i in range(NQ):
            kv_proj(i)
        for i in range(1, NQ):
            q_proj(i)

    @pl.when((step < H - 1) & ((step & 1) == 1))
    def _next_weights():
        pair = (step + 1) >> 1
        for cp in w_copies(pair):
            cp.wait()

        @pl.when(pair + 1 < H // 2)
        def _():
            for cp in w_copies(pair + 1):
                cp.start()

    def attention(h, project_next):
        rows = S // H
        r0 = pl.multiple_of(h * rows, rows)
        xg = x_ref[pl.ds(r0, rows), :].astype(jnp.float32) * gw_ref[...].astype(jnp.float32)
        gl = jnp.sum(xg, axis=-1, keepdims=True)
        g_s[pl.ds(r0, rows), :] = jnp.broadcast_to(jax.nn.sigmoid(gl), (rows, CG))

        hb = BQ // 2
        row = lax.broadcasted_iota(jnp.int32, (hb, hb), 0)
        col = lax.broadcasted_iota(jnp.int32, (hb, hb), 1)
        tri = col <= row
        neg = -1e9 * LOG2E
        for i in reversed(range(NQ)):
            r0, r1, r2 = i * BQ, i * BQ + hb, (i + 1) * BQ
            s = lax.dot_general(q_s[r0:r2, :], k_s[:r1, :], NT, preferred_element_type=jnp.float32)
            sl = lax.dot_general(q_s[r1:r2, :], k_s[r1:r2, :], NT, preferred_element_type=jnp.float32)
            if i == NQ - 1:
                q_proj(0)
                if project_next:
                    unpack_q(h + 1)
                    unpack_kv(h + 1)
            elif project_next:
                kv_proj(i + 1)
                q_proj(i + 1)
            st = jnp.where(tri, s[:hb, r0:], neg)
            if i > 0:
                st = jnp.concatenate([s[:hb, :r0], st], axis=1)
            sb = jnp.concatenate([s[hb:], jnp.where(tri, sl, neg)], axis=1)
            pt = jnp.exp2(st - jnp.max(st, axis=-1, keepdims=True))
            pb = jnp.exp2(sb - jnp.max(sb, axis=-1, keepdims=True))
            lt = jnp.sum(pt, axis=-1, keepdims=True)
            lb = jnp.sum(pb, axis=-1, keepdims=True)
            pt = pt.astype(jnp.bfloat16)
            pb = pb.astype(jnp.bfloat16)
            o = jnp.dot(jnp.concatenate([pt, pb[:, :r1]], axis=0), v_s[:r1, :],
                        preferred_element_type=jnp.float32)
            ol = jnp.dot(pb[:, r1:], v_s[r1:r2, :], preferred_element_type=jnp.float32)
            ctx_s[h, r0:r1, :] = (o[:hb] / lt).astype(jnp.bfloat16)
            ctx_s[h, r1:r2, :] = ((o[hb:] + ol) / lb).astype(jnp.bfloat16)
        if project_next:
            kv_proj(0)

    @pl.when(step < H - 1)
    def _heads():
        attention(step, True)

    @pl.when(step == H - 1)
    def _last_head():
        attention(step, False)

    @pl.when(step >= H)
    def _mix():
        def out_proj(j):
            r = slice(j * CB, (j + 1) * CB)
            lhs = jnp.concatenate([ctx_s[hh, r, :] for hh in range(H)], axis=1)
            b = jnp.dot(lhs, wo_ref[...], preferred_element_type=jnp.float32)
            b_s[r, :] = (1.0 - g_s[r, :]) * b

        kp_s[0:8, :] = jnp.zeros((8, CG), jnp.float32)
        kp_s[8:, :] = ak_ref[...].astype(jnp.float32)
        sk = sk_ref[...].astype(jnp.float32)
        fwd = fwd_ref[...]
        out_proj(0)
        for i in range(NB):
            acc = kp_s[8 + i * CB:8 + (i + 1) * CB, :] * sk[0:1, :]
            for t in range(1, 4):
                acc = acc + kp_s[8 - t + i * CB:8 - t + (i + 1) * CB, :] * sk[t:t + 1, :]
            kvb = (acc * av_ref[i * CB:(i + 1) * CB, :].astype(jnp.float32)).astype(jnp.bfloat16)
            kv_s[i * CB:(i + 1) * CB, :] = kvb
            xf_s[i] = jnp.dot(fwd, kvb, preferred_element_type=jnp.float32)
        out_proj(1)
        hq = CB // 2
        prev = None
        for m in range(NB):
            hf = lax.dot_general(fwd, hk_ref[:, m * CB:(m + 1) * CB], NT,
                                 preferred_element_type=jnp.float32)
            if prev is None:
                hf_s[m] = hf
            else:
                hf_s[m, 0:hq, :] = hf[0:hq] - prev[2 * hq:3 * hq]
                hf_s[m, hq:2 * hq, :] = hf[hq:2 * hq] + prev[3 * hq:4 * hq]
                hf_s[m, 2 * hq:3 * hq, :] = hf[2 * hq:3 * hq] + prev[0:hq]
                hf_s[m, 3 * hq:4 * hq, :] = hf[3 * hq:4 * hq] - prev[hq:2 * hq]
            prev = hf
        TI = 4
        nchunk = CB // 16
        for fc in range(nchunk):
            for half in range(2):
                f0 = fc * 16 + half * 8
                re = slice(f0, f0 + 8)
                im = slice(CB + f0, CB + f0 + 8)
                for i0 in range(0, NB, TI):
                    ar = [None] * TI
                    ai = [None] * TI
                    for m in range(i0 + TI):
                        gr = hf_s[m, re, :]
                        gi = hf_s[m, im, :]
                        for u in range(TI):
                            d = i0 + u - m
                            if d < 0:
                                continue
                            xr = xf_s[d, re, :]
                            xi = xf_s[d, im, :]
                            pr = gr * xr - gi * xi
                            pi = gr * xi + gi * xr
                            ar[u] = pr if ar[u] is None else ar[u] + pr
                            ai[u] = pi if ai[u] is None else ai[u] + pi
                    for u in range(TI):
                        z_s[i0 + u, re, :] = ar[u]
                        z_s[i0 + u, im, :] = ai[u]
            if fc < nchunk - 1:
                out_proj(2 + 2 * fc)
                out_proj(3 + 2 * fc)
        inv = inv_ref[...]
        sd = sd_ref[...].astype(jnp.float32)
        for i in range(NB):
            r = slice(i * CB, (i + 1) * CB)
            y = jnp.dot(inv, z_s[i].astype(jnp.bfloat16), preferred_element_type=jnp.float32)
            a = xq_ref[r, :].astype(jnp.float32) * (y + kv_s[r, :].astype(jnp.float32) * sd)
            o_ref[r, :] = (g_s[r, :] * a + b_s[r, :]).astype(o_ref.dtype)


@jax.jit
def pallas_gated_mix__ssm_conv_h3__compressed_kv_cla__prompt_kernel(
    A_q: jax.Array,
    A_k: jax.Array,
    A_v: jax.Array,
    A_shift_k: jax.Array,
    A_ssm_k: jax.Array,
    A_ssm_D: jax.Array,
    B_x: jax.Array,
    B_c_kv: jax.Array,
    B_w_q: jax.Array,
    B_w_uk: jax.Array,
    B_w_uv: jax.Array,
    B_w_o: jax.Array,
    gate_w: jax.Array,
):
    del B_x
    x = A_q.reshape(S, DM)
    fwd = jnp.asarray(_FWD_NP, dtype=jnp.bfloat16)
    inv = jnp.asarray(_INV_NP, dtype=jnp.bfloat16)

    one = pl.Buffered(1)

    def whole(shape):
        return pl.BlockSpec(shape, lambda s: (0,) * len(shape), pipeline_mode=one)

    def grp(s):
        return jnp.maximum(s - H, 0)

    col = lambda rows: pl.BlockSpec((rows, CG), lambda s: (0, grp(s)))

    out = pl.pallas_call(
        _kernel,
        grid=(H + NG,),
        in_specs=[
            whole((S, DM)),
            whole((S, DC)),
            pl.BlockSpec(memory_space=pl.ANY),
            pl.BlockSpec(memory_space=pl.ANY),
            pl.BlockSpec(memory_space=pl.ANY),
            whole((1, DM)),
            whole((2 * CB, CB)),
            whole((CB, 2 * CB)),
            col(S),
            col(S),
            col(S),
            col(4),
            pl.BlockSpec((CG, S), lambda s: (grp(s), 0)),
            col(1),
            col(H * HD),
        ],
        out_specs=col(S),
        out_shape=jax.ShapeDtypeStruct((S, DM), jnp.bfloat16),
        scratch_shapes=[
            pltpu.VMEM((S, HD), jnp.bfloat16),
            pltpu.VMEM((S, HD), jnp.bfloat16),
            pltpu.VMEM((S, HD), jnp.bfloat16),
            pltpu.VMEM((H, S, HD), jnp.bfloat16),
            pltpu.VMEM((S, CG), jnp.float32),
            pltpu.VMEM((S + 8, CG), jnp.float32),
            pltpu.VMEM((NB, 2 * CB, CG), jnp.float32),
            pltpu.VMEM((NB, 2 * CB, CG), jnp.float32),
            pltpu.VMEM((NB, 2 * CB, CG), jnp.float32),
            pltpu.VMEM((S, CG), jnp.float32),
            pltpu.VMEM((S, CG), jnp.bfloat16),
            pltpu.VMEM((2, DM, HD), jnp.uint32),
            pltpu.VMEM((2, DC, HD), jnp.uint32),
            pltpu.VMEM((2, DC, HD), jnp.uint32),
            pltpu.VMEM((DM, HD), jnp.bfloat16),
            pltpu.VMEM((DC, 2 * HD), jnp.bfloat16),
            pltpu.SemaphoreType.DMA((3, 2)),
        ],
        compiler_params=pltpu.CompilerParams(
            dimension_semantics=("arbitrary",),
            vmem_limit_bytes=110 * 1024 * 1024,
        ),
    )(
        x,
        B_c_kv.reshape(S, DC),
        B_w_q,
        B_w_uk,
        B_w_uv,
        gate_w.reshape(1, DM),
        fwd,
        inv,
        x,
        A_k.reshape(S, DM),
        A_v.reshape(S, DM),
        A_shift_k.T,
        A_ssm_k,
        A_ssm_D.reshape(1, DM),
        B_w_o.reshape(H * HD, DM),
    )
    return out.reshape(1, S, DM)
```

```python
import functools

import numpy as np

import jax
import jax.numpy as jnp
from jax import lax
import jax.experimental.pallas as pl
import jax.experimental.pallas.tpu as pltpu

S = 2048
DM = 1024
H = 32
HD = 128
DC = 512
L = 128
CB = 128
NB = S // CB
NG = DM // L
BQ = 256
NQ = S // BQ
LAG = 2
WLAG = 2
GS = 4

LOG2E = 1.4426950408889634
NN = (((1,), (0,)), ((), ()))
NT = (((1,), (1,)), ((), ()))
F32 = jnp.float32
BF16 = jnp.bfloat16
U32 = jnp.uint32


def _dft_matrices():
    n = 2 * CB
    f = np.concatenate([np.arange(0, CB, 2), np.arange(1, CB, 2)]).astype(np.float64)
    j = np.arange(CB, dtype=np.float64)
    ang = 2.0 * np.pi * np.outer(f + 0.5, j) / n
    fwd = np.concatenate([np.cos(ang), -np.sin(ang)], axis=0)
    inv = np.concatenate([np.cos(ang).T, -np.sin(ang).T], axis=1)
    inv = inv * (2.0 / n)
    return fwd.astype(np.float32), inv.astype(np.float32)


_FWD_NP, _INV_NP = _dft_matrices()


def _unpack(w):
    return pltpu.bitcast(w, BF16)


def _rows(r0, r1):
    return slice(r0 // 2, r1 // 2)


def _head_weight(w32, h):
    sh = (16 - 16 * (h & 1)).astype(U32)
    return pltpu.bitcast((w32 << sh) & U32(0xFFFF0000), F32)


def _kernel(x_hbm, c_hbm, wq_hbm, wuk_hbm, wuv_hbm, ak_hbm, av_hbm, hk_hbm, wo_hbm,
            gw_ref, sk_ref, sd_ref, fwd_ref, inv_ref,
            o_hbm,
            x_s, c_s, q_s, k_s, v_s, ctx_s, g_s, wq_b, wuk_b, wuv_b, wq_s, wkv_s,
            ak_b, av_b, hk_b, wo_b, o_b, kp_s, xf_s, hf_s, z_s, b_s, kv_s,
            xsem, csem, wsem, gsem, osem):

    q_w, k_w, v_w, ctx_w, wq_w, wkv_w, kv_w = (
        r.bitcast(U32) for r in (q_s, k_s, v_s, ctx_s, wq_s, wkv_s, kv_s))

    def col_copies(src, dst, sem):
        return [pltpu.make_async_copy(src.bitcast(U32).at[:, pl.ds(n * L, L)], dst.at[n], sem.at[n])
                for n in range(dst.shape[0])]

    def w_copies(pair):
        slot = pair & 1
        return [
            pltpu.make_async_copy(src.bitcast(U32).at[:, pair, :], dst.at[slot], wsem.at[n, slot])
            for n, (src, dst) in enumerate(((wq_hbm, wq_b), (wuk_hbm, wuk_b), (wuv_hbm, wuv_b)))
        ]

    def g_copies(g):
        slot = g & 1
        cols = pl.ds(pl.multiple_of(g * L, L), L)
        chans = pl.ds(pl.multiple_of(g * (L // 2), L // 2), L // 2)
        srcs = (ak_hbm.bitcast(U32).at[:, cols], av_hbm.bitcast(U32).at[:, cols],
                hk_hbm.bitcast(U32).at[chans, :], wo_hbm.bitcast(U32).at[:, cols])
        return [pltpu.make_async_copy(src, dst.at[slot], gsem.at[n, slot])
                for n, (src, dst) in enumerate(zip(srcs, (ak_b, av_b, hk_b, wo_b)))]

    def o_copy(g):
        slot = g & 1
        return pltpu.make_async_copy(
            o_b.at[slot], o_hbm.at[:, pl.ds(pl.multiple_of(g * L, L), L)], osem.at[slot])

    def unpack_q(h):
        wq_s[...] = _head_weight(wq_b[(h >> 1) & 1], h).astype(BF16)

    def unpack_kv(h):
        slot = (h >> 1) & 1
        wkv_s[0] = _head_weight(wuk_b[slot], h).astype(BF16)
        wkv_s[1] = _head_weight(wuv_b[slot], h).astype(BF16)

    def wide(ref, rows, tiles):
        return jnp.concatenate([_unpack(ref[n, rows, :]) for n in tiles], axis=1)

    def attention(h, first=False, project_next=True):
        st = {"deps": []}
        hb = BQ // 2
        row = lax.broadcasted_iota(jnp.int32, (hb, hb), 0)
        col = lax.broadcasted_iota(jnp.int32, (hb, hb), 1)
        tri = col <= row
        neg = -1e9 * LOG2E
        never = row > h + 2 * S
        never8 = never[:8]

        def gated(w32):
            if len(st["deps"]) >= WLAG:
                dep = st["deps"][-WLAG]
                parts = []
                for r in range(0, w32.shape[0], L // 2):
                    parts += [jnp.where(never8, dep, w32[r:r + 8]), w32[r + 8:r + L // 2]]
                w32 = jnp.concatenate(parts, axis=0)
            return _unpack(w32)

        def mark(y):
            st["deps"].append(pltpu.bitcast(y[:8, :L], U32))
            return y

        def groups(i):
            nt = 2 * i + 1
            return [(j, min(j + GS, nt)) for j in range(0, nt, GS)]

        def qk(i, g):
            r0, r1, r2 = i * BQ, i * BQ + hb, (i + 1) * BQ
            j0, j1 = groups(i)[g]
            d = st.setdefault(i, dict(t=[], b=[], acc=[None, None], o=None))
            kk = gated(k_w[_rows(j0 * hb, j1 * hb), :])
            s = lax.dot_general(_unpack(q_w[_rows(r0, r2), :]), kk, NT, preferred_element_type=F32)
            for j in range(j1 - j0):
                d["t"].append(s[:hb, j * hb:(j + 1) * hb])
                d["b"].append(s[hb:, j * hb:(j + 1) * hb])
            if g == len(groups(i)) - 1:
                kl = gated(k_w[_rows(r1, r2), :])
                sl = lax.dot_general(_unpack(q_w[_rows(r1, r2), :]), kl, NT, preferred_element_type=F32)
                d["t"][-1] = jnp.where(tri, d["t"][-1], neg)
                d["b"].append(jnp.where(tri, sl, neg))
                d["m"] = [jnp.max(functools.reduce(jnp.maximum, tiles), axis=-1, keepdims=True)
                          for tiles in (d["t"], d["b"])]
            if j1 - j0 >= 3:
                mark(s)

        def pv(i, g):
            r0, r1, r2 = i * BQ, i * BQ + hb, (i + 1) * BQ
            j0, j1 = groups(i)[g]
            d = st[i]
            last = g == len(groups(i)) - 1
            ps = []
            for half, tiles in enumerate((d["t"], d["b"])):
                tl = tiles[j0:] if last else tiles[j0:j1]
                acc = d["acc"][half]
                m = d["m"][half]
                if g > 0:
                    dep = pltpu.bitcast(st["deps"][-LAG], F32)
                    m = jnp.where(never, jnp.concatenate([dep] * (hb // 8), axis=0), m)
                out = []
                for j, t in enumerate(tl):
                    p = jnp.exp2(t - m)
                    acc = p if acc is None else acc + p
                    if j == len(tl) - 1:
                        if acc is not p:
                            p = jnp.where(never, acc, p)
                        if last and (i + 1) in st:
                            p = jnp.where(never, st[i + 1]["out"][half], p)
                    out.append(p)
                d["acc"][half] = acc
                ps.append(out)
            lhs = jnp.concatenate([jnp.concatenate(ps[0], axis=1),
                                   jnp.concatenate(ps[1][:j1 - j0], axis=1)], axis=0).astype(BF16)
            vv = gated(v_w[_rows(j0 * hb, j1 * hb), :])
            o = jnp.dot(lhs, vv, preferred_element_type=F32)
            d["o"] = o if d["o"] is None else d["o"] + o
            if last:
                vl = gated(v_w[_rows(r1, r2), :])
                ol = jnp.dot(ps[1][-1].astype(BF16), vl, preferred_element_type=F32)
                lt, lb = [jnp.sum(a, axis=-1, keepdims=True) for a in d["acc"]]
                d["out"] = (d["o"][:hb] / lt, (d["o"][hb:] + ol) / lb)
                ctx_s[h, r0:r1, :] = d["out"][0].astype(BF16)
                ctx_s[h, r1:r2, :] = d["out"][1].astype(BF16)
            if j1 - j0 >= 3:
                mark(o)

        def qp(i, half):
            r = _rows(i * BQ, (i + 1) * BQ)
            w = gated(wq_w[_rows(half * DM // 2, (half + 1) * DM // 2), :])
            q = mark(jnp.dot(wide(x_s, r, range(half * NG // 2, (half + 1) * NG // 2)), w,
                             preferred_element_type=F32))
            if half == 0:
                st["q", i] = q
            else:
                q_s[i * BQ:(i + 1) * BQ, :] = ((st["q", i] + q) * (HD ** -0.5 * LOG2E)).astype(BF16)

        def kvp(i, which):
            r = _rows(i * BQ, (i + 1) * BQ)
            w = gated(wkv_w[which])
            y = mark(jnp.dot(wide(c_s, r, range(DC // L)), w, preferred_element_type=F32))
            (k_s, v_s)[which][i * BQ:(i + 1) * BQ, :] = y.astype(BF16)

        def Q(*js):
            return [functools.partial(qp, j, half) for j in js for half in range(2)]

        def KV(*js):
            return [functools.partial(kvp, j, w) for j in js for w in range(2)] if project_next else []

        if first:
            for cp in col_copies(c_hbm, c_s, csem) + w_copies(0)[1:]:
                cp.wait()
            unpack_kv(h)
            for u in KV(*range(NQ)):
                u()
            for cp in col_copies(x_hbm, x_s, xsem) + w_copies(0)[:1]:
                cp.wait()
            unpack_q(h)
            for u in Q(NQ - 1):
                u()
            return

        rows = S // H
        xr = pl.ds(pl.multiple_of(h * (rows // 2), rows // 2), rows // 2)
        gw = gw_ref[...].astype(F32)
        gl = functools.reduce(jnp.add, [
            _unpack(x_s[n, xr, :]).astype(F32) * gw[:, n * L:(n + 1) * L] for n in range(NG)])
        gl = jnp.sum(gl, axis=-1, keepdims=True)
        g_s[pl.ds(pl.multiple_of(h * rows, rows), rows), :] = jnp.broadcast_to(
            jax.nn.sigmoid(gl), (rows, L))

        QN = ([lambda: unpack_q(h + 1)] + Q(NQ - 1)) if project_next else []
        UK = [lambda: unpack_kv(h + 1)] if project_next else []
        fill = {7: Q(6), 6: Q(5, 4, 3), 5: UK + Q(2, 1) + KV(7), 4: Q(0) + QN + KV(6),
                3: KV(5), 2: KV(4), 1: KV(3), 0: KV(2), -1: KV(1, 0)}

        def spread(*seqs):
            keyed = [((n + 0.5) / len(q) + 1e-3 * k, u) for k, q in enumerate(seqs) for n, u in enumerate(q)]
            return [u for _, u in sorted(keyed, key=lambda t: t[0])]

        for i in range(NQ - 1, -2, -1):
            a = [functools.partial(qk, i, g) for g in range(len(groups(i)))] if i >= 0 else []
            b = [functools.partial(pv, i + 1, g) for g in range(len(groups(i + 1)))] if i + 1 < NQ else []
            units = (a + fill[i]) if i == NQ - 1 else spread(a, fill[i], b)
            for u in units:
                u()

    def head_step(h, carry):
        @pl.when((h & 1) == 1)
        def _next_weights():
            pair = (h + 1) >> 1
            for cp in w_copies(pair):
                cp.wait()

            @pl.when(pair + 1 < H // 2)
            def _():
                for cp in w_copies(pair + 1):
                    cp.start()

        attention(h)
        return carry

    def mix_step(g, carry):
        slot = g & 1
        for cp in g_copies(g):
            cp.wait()

        @pl.when(g + 1 < NG)
        def _():
            for cp in g_copies(g + 1):
                cp.start()

        @pl.when(g >= 2)
        def _():
            o_copy(g - 2).wait()

        cols = pl.ds(pl.multiple_of(g * L, L), L)

        def out_proj(j):
            r = slice(j * CB, (j + 1) * CB)
            lhs = wide(ctx_w, _rows(j * CB, (j + 1) * CB), range(H))
            b = jnp.dot(lhs, _unpack(wo_b[slot]), preferred_element_type=F32)
            b_s[r, :] = (1.0 - g_s[r, :]) * b

        kp_s[0:8, :] = jnp.zeros((8, L), F32)
        kp_s[8:, :] = _unpack(ak_b[slot]).astype(F32)
        sk = sk_ref[:, cols].astype(F32)
        fwd = fwd_ref[...]
        out_proj(0)
        for i in range(NB):
            acc = kp_s[8 + i * CB:8 + (i + 1) * CB, :] * sk[0:1, :]
            for t in range(1, 4):
                acc = acc + kp_s[8 - t + i * CB:8 - t + (i + 1) * CB, :] * sk[t:t + 1, :]
            kvb = (acc * _unpack(av_b[slot, _rows(i * CB, (i + 1) * CB), :]).astype(F32)).astype(BF16)
            kv_s[i * CB:(i + 1) * CB, :] = kvb
            xf_s[i] = jnp.dot(fwd, kvb, preferred_element_type=F32)
        out_proj(1)
        hq = CB // 2
        prev = None
        for m in range(NB):
            hf = lax.dot_general(fwd, _unpack(hk_b[slot, :, m * CB:(m + 1) * CB]), NT,
                                 preferred_element_type=F32)
            if prev is None:
                hf_s[m] = hf
            else:
                hf_s[m, 0:hq, :] = hf[0:hq] - prev[2 * hq:3 * hq]
                hf_s[m, hq:2 * hq, :] = hf[hq:2 * hq] + prev[3 * hq:4 * hq]
                hf_s[m, 2 * hq:3 * hq, :] = hf[2 * hq:3 * hq] + prev[0:hq]
                hf_s[m, 3 * hq:4 * hq, :] = hf[3 * hq:4 * hq] - prev[hq:2 * hq]
            prev = hf
        TI = 4
        nchunk = CB // 16
        for fc in range(nchunk):
            for half in range(2):
                f0 = fc * 16 + half * 8
                re = slice(f0, f0 + 8)
                im = slice(CB + f0, CB + f0 + 8)
                for i0 in range(0, NB, TI):
                    ar = [None] * TI
                    ai = [None] * TI
                    for m in range(i0 + TI):
                        gr = hf_s[m, re, :]
                        gi = hf_s[m, im, :]
                        for u in range(TI):
                            d = i0 + u - m
                            if d < 0:
                                continue
                            xr = xf_s[d, re, :]
                            xi = xf_s[d, im, :]
                            pr = gr * xr - gi * xi
                            pi = gr * xi + gi * xr
                            ar[u] = pr if ar[u] is None else ar[u] + pr
                            ai[u] = pi if ai[u] is None else ai[u] + pi
                    for u in range(TI):
                        z_s[i0 + u, re, :] = ar[u]
                        z_s[i0 + u, im, :] = ai[u]
            if fc < nchunk - 1:
                out_proj(2 + 2 * fc)
                out_proj(3 + 2 * fc)
        inv = inv_ref[...]
        sd = sd_ref[:, cols].astype(F32)
        for i in range(NB):
            r = slice(i * CB, (i + 1) * CB)
            rw = _rows(i * CB, (i + 1) * CB)
            y = jnp.dot(inv, z_s[i].astype(BF16), preferred_element_type=F32)
            a = _unpack(x_s[g, rw, :]).astype(F32) * (y + _unpack(kv_w[rw, :]).astype(F32) * sd)
            o_b[slot, r, :] = (g_s[r, :] * a + b_s[r, :]).astype(BF16)
        o_copy(g).start()
        return carry

    zero = jnp.int32(0)
    first = (col_copies(c_hbm, c_s, csem) + w_copies(0)[1:] + col_copies(x_hbm, x_s, xsem)
             + w_copies(0)[:1] + w_copies(1) + g_copies(0))
    for cp in first:
        cp.start()
    attention(zero, first=True)
    lax.fori_loop(0, H - 1, head_step, 0)
    attention(zero + (H - 1), project_next=False)
    lax.fori_loop(0, NG, mix_step, 0)
    o_copy(NG - 2).wait()
    o_copy(NG - 1).wait()


@jax.jit
def pallas_gated_mix__ssm_conv_h3__compressed_kv_cla__prompt_kernel(
    A_q: jax.Array,
    A_k: jax.Array,
    A_v: jax.Array,
    A_shift_k: jax.Array,
    A_ssm_k: jax.Array,
    A_ssm_D: jax.Array,
    B_x: jax.Array,
    B_c_kv: jax.Array,
    B_w_q: jax.Array,
    B_w_uk: jax.Array,
    B_w_uv: jax.Array,
    B_w_o: jax.Array,
    gate_w: jax.Array,
):
    del B_x
    hbm = pl.BlockSpec(memory_space=pl.ANY)
    vmem = pl.BlockSpec(memory_space=pltpu.VMEM)
    out = pl.pallas_call(
        _kernel,
        in_specs=[hbm] * 9 + [vmem] * 5,
        out_specs=hbm,
        out_shape=jax.ShapeDtypeStruct((S, DM), BF16),
        scratch_shapes=[
            pltpu.VMEM((NG, S // 2, L), U32),
            pltpu.VMEM((DC // L, S // 2, L), U32),
            pltpu.VMEM((S, HD), BF16),
            pltpu.VMEM((S, HD), BF16),
            pltpu.VMEM((S, HD), BF16),
            pltpu.VMEM((H, S, HD), BF16),
            pltpu.VMEM((S, L), F32),
            pltpu.VMEM((2, DM, HD), U32),
            pltpu.VMEM((2, DC, HD), U32),
            pltpu.VMEM((2, DC, HD), U32),
            pltpu.VMEM((DM, HD), BF16),
            pltpu.VMEM((2, DC, HD), BF16),
            pltpu.VMEM((2, S // 2, L), U32),
            pltpu.VMEM((2, S // 2, L), U32),
            pltpu.VMEM((2, L // 2, S), U32),
            pltpu.VMEM((2, H * HD // 2, L), U32),
            pltpu.VMEM((2, S, L), BF16),
            pltpu.VMEM((S + 8, L), F32),
            pltpu.VMEM((NB, 2 * CB, L), F32),
            pltpu.VMEM((NB, 2 * CB, L), F32),
            pltpu.VMEM((NB, 2 * CB, L), F32),
            pltpu.VMEM((S, L), F32),
            pltpu.VMEM((S, L), BF16),
            pltpu.SemaphoreType.DMA((NG,)),
            pltpu.SemaphoreType.DMA((DC // L,)),
            pltpu.SemaphoreType.DMA((3, 2)),
            pltpu.SemaphoreType.DMA((4, 2)),
            pltpu.SemaphoreType.DMA((2,)),
        ],
        compiler_params=pltpu.CompilerParams(vmem_limit_bytes=110 * 1024 * 1024),
    )(
        A_q.reshape(S, DM),
        B_c_kv.reshape(S, DC),
        B_w_q,
        B_w_uk,
        B_w_uv,
        A_k.reshape(S, DM),
        A_v.reshape(S, DM),
        A_ssm_k,
        B_w_o.reshape(H * HD, DM),
        gate_w.reshape(1, DM),
        A_shift_k.T,
        A_ssm_D.reshape(1, DM),
        jnp.asarray(_FWD_NP, dtype=BF16),
        jnp.asarray(_INV_NP, dtype=BF16),
    )
    return out.reshape(1, S, DM)
```

```python
import functools

import numpy as np

import jax
import jax.numpy as jnp
from jax import lax
import jax.experimental.pallas as pl
import jax.experimental.pallas.tpu as pltpu

S = 2048
DM = 1024
H = 32
HD = 128
DC = 512
L = 128
CB = 128
NB = S // CB
NG = DM // L
BQ = 256
NQ = S // BQ
LAG = 2
HP = 4
TI = 4
TAIL = 4
N1 = 2
N2 = 3
N3 = 14
GS = 4

LOG2E = 1.4426950408889634
NN = (((1,), (0,)), ((), ()))
NT = (((1,), (1,)), ((), ()))
F32 = jnp.float32
BF16 = jnp.bfloat16
U32 = jnp.uint32


def _dft_matrices():
    n = 2 * CB
    f = np.concatenate([np.arange(0, CB, 2), np.arange(1, CB, 2)]).astype(np.float64)
    j = np.arange(CB, dtype=np.float64)
    ang = 2.0 * np.pi * np.outer(f + 0.5, j) / n
    fwd = np.concatenate([np.cos(ang), -np.sin(ang)], axis=0)
    inv = np.concatenate([np.cos(ang).T, -np.sin(ang).T], axis=1)
    inv = inv * (2.0 / n)
    return fwd.astype(np.float32).astype(BF16), inv.astype(np.float32).astype(BF16)


_FWD_NP, _INV_NP = _dft_matrices()


def _unpack(w):
    return pltpu.bitcast(w, BF16)


def _rows(r0, r1):
    return slice(r0 // 2, r1 // 2)


def _head_weight(w32, h):
    sh = (16 - 16 * (h & 1)).astype(U32)
    return pltpu.bitcast((w32 << sh) & U32(0xFFFF0000), F32)


class _Order:
    def __init__(self, dft_ref):
        self.never = dft_ref[0:16, :].astype(F32)[0:1, :] > 2.0
        self.marks = []

    def mark(self, y):
        self.marks.append(y)
        return y

    def tie(self, a, lag, frac=0.0):
        if len(self.marks) < lag:
            return a
        y = self.marks[-lag]
        r = int(frac * (y.shape[0] // 8)) * 8
        dep = y[r:r + 8, :L]
        if a.dtype == U32:
            dep = pltpu.bitcast(dep, U32)
        n = a.shape[0]
        return jnp.where(self.never, jnp.concatenate([dep] * (n // 8), axis=0), a)

    def trickle(self, a, lag, r0):
        return jnp.where(self.never, self.marks[-lag][r0:r0 + L, :L], a)

    def weights(self, w32, lag=2):
        rows = []
        for r in range(0, w32.shape[0], L // 2):
            head = [self.tie(w32[r:r + 8, c:c + L], lag) for c in range(0, w32.shape[1], L)]
            rows += [jnp.concatenate(head, axis=1), w32[r + 8:r + L // 2]]
        return _unpack(jnp.concatenate(rows, axis=0))


def _spread(*seqs):
    keyed = [((n + 0.5) / len(q) + 1e-3 * k, u) for k, q in enumerate(seqs) for n, u in enumerate(q)]
    return [u for _, u in sorted(keyed, key=lambda t: t[0])]


def _kernel(x_hbm, c_hbm, wq_hbm, wuk_hbm, wuv_hbm, ak_hbm, av_hbm, hk_hbm, wo_hbm,
            gw_ref, sk_ref, sd_ref, fwd_ref, inv_ref,
            o_hbm,
            x_s, c_s, q_s, k_s, v_s, ctx_s, g_s, wq_b, wuk_b, wuv_b, wq_s, wkv_s,
            ak_b, av_b, hk_b, wo_b, o_b, sd_s, kp_s, xf_s, hf_s, z_s, b_s, kv_s,
            xsem, csem, wsem, gsem, osem):

    q_w, k_w, v_w, ctx_w, wq_w, wkv_w, kv_w = (
        r.bitcast(U32) for r in (q_s, k_s, v_s, ctx_s, wq_s, wkv_s, kv_s))

    def row_copy(src, dst, sem, i):
        r = pl.ds(i * BQ // 2, BQ // 2)
        return pltpu.make_async_copy(src.bitcast(U32).at[r, :], dst.at[r, :], sem.at[i])

    def w_copy(n, pair):
        src, dst = ((wq_hbm, wq_b), (wuk_hbm, wuk_b), (wuv_hbm, wuv_b))[n]
        slot = pair & 1
        return pltpu.make_async_copy(src.bitcast(U32).at[:, pair, :], dst.at[slot], wsem.at[n, slot])

    def g_copies(g):
        slot = g & 1
        cols = pl.ds(pl.multiple_of(g * L, L), L)
        chans = pl.ds(pl.multiple_of(g * (L // 2), L // 2), L // 2)
        srcs = (ak_hbm.bitcast(U32).at[:, cols], av_hbm.bitcast(U32).at[:, cols],
                hk_hbm.bitcast(U32).at[chans, :], wo_hbm.bitcast(U32).at[:, cols])
        return [pltpu.make_async_copy(src, dst.at[slot], gsem.at[n, slot])
                for n, (src, dst) in enumerate(zip(srcs, (ak_b, av_b, hk_b, wo_b)))]

    def o_copy(g):
        slot = g & 1
        return pltpu.make_async_copy(
            o_b.at[slot], o_hbm.at[:, pl.ds(pl.multiple_of(g * L, L), L)], osem.at[slot])

    def unpack_q(h):
        wq_s[...] = _head_weight(wq_b[(h >> 1) & 1], h).astype(BF16)

    def unpack_kv(h):
        slot = (h >> 1) & 1
        wkv_s[0] = _head_weight(wuk_b[slot], h).astype(BF16)
        wkv_s[1] = _head_weight(wuv_b[slot], h).astype(BF16)

    def wide(ref, rows, tiles):
        return jnp.concatenate([_unpack(ref[n, rows, :]) for n in tiles], axis=1)

    def attention(h, order, prologue=False, project_next=True):
        st = {}
        hb = BQ // 2
        row = lax.broadcasted_iota(jnp.int32, (hb, hb), 0)
        col = lax.broadcasted_iota(jnp.int32, (hb, hb), 1)
        tri = col <= row
        neg = -1e9 * LOG2E
        never, gated, mark = order.never, order.weights, order.mark

        def groups(i):
            nt = 2 * i + 1
            return [(j, min(j + GS, nt)) for j in range(0, nt, GS)]

        def qk(i, g):
            r0, r1, r2 = i * BQ, i * BQ + hb, (i + 1) * BQ
            j0, j1 = groups(i)[g]
            d = st.setdefault(i, dict(t={}, b={}, acc=[None, None], o=None, n=0))
            kk = gated(k_w[_rows(j0 * hb, j1 * hb), :])
            s = lax.dot_general(_unpack(q_w[_rows(r0, r2), :]), kk, NT, preferred_element_type=F32)
            for j in range(j1 - j0):
                d["t"][j0 + j] = s[:hb, j * hb:(j + 1) * hb]
                d["b"][j0 + j] = s[hb:, j * hb:(j + 1) * hb]
            if g == len(groups(i)) - 1:
                kl = gated(k_w[_rows(r1, r2), :])
                sl = lax.dot_general(_unpack(q_w[_rows(r1, r2), :]), kl, NT, preferred_element_type=F32)
                d["t"][j1 - 1] = jnp.where(tri, d["t"][j1 - 1], neg)
                d["b"][j1] = jnp.where(tri, sl, neg)
            d["n"] += 1
            if d["n"] == len(groups(i)):
                d["t"], d["b"] = ([t[j] for j in sorted(t)] for t in (d["t"], d["b"]))
                d["m"] = [jnp.max(functools.reduce(jnp.maximum, tiles), axis=-1, keepdims=True)
                          for tiles in (d["t"], d["b"])]
            if j1 - j0 >= 3:
                mark(s)

        def pv(i, g):
            r0, r1, r2 = i * BQ, i * BQ + hb, (i + 1) * BQ
            j0, j1 = groups(i)[g]
            d = st[i]
            last = g == len(groups(i)) - 1
            ps = []
            for half, tiles in enumerate((d["t"], d["b"])):
                tl = tiles[j0:] if last else tiles[j0:j1]
                acc = d["acc"][half]
                m = d["m"][half]
                if g > 0:
                    m = order.trickle(m, LAG, half * hb)
                out = []
                for j, t in enumerate(tl):
                    p = jnp.exp2(t - m)
                    acc = p if acc is None else acc + p
                    if j == len(tl) - 1:
                        if acc is not p:
                            p = jnp.where(never, acc, p)
                        if last and (i + 1) in st:
                            p = jnp.where(never, st[i + 1]["out"][half], p)
                    out.append(p)
                d["acc"][half] = acc
                ps.append(out)
            lhs = jnp.concatenate([jnp.concatenate(ps[0], axis=1),
                                   jnp.concatenate(ps[1][:j1 - j0], axis=1)], axis=0).astype(BF16)
            vv = gated(v_w[_rows(j0 * hb, j1 * hb), :])
            o = jnp.dot(lhs, vv, preferred_element_type=F32)
            d["o"] = o if d["o"] is None else d["o"] + o
            if last:
                vl = gated(v_w[_rows(r1, r2), :])
                ol = jnp.dot(ps[1][-1].astype(BF16), vl, preferred_element_type=F32)
                lt, lb = [jnp.sum(a, axis=-1, keepdims=True) for a in d["acc"]]
                d["out"] = (d["o"][:hb] / lt, (d["o"][hb:] + ol) / lb)
                ctx_s[h, r0:r1, :] = d["out"][0].astype(BF16)
                ctx_s[h, r1:r2, :] = d["out"][1].astype(BF16)
            if j1 - j0 >= 3:
                mark(o)

        def qp(i, half):
            r = _rows(i * BQ, (i + 1) * BQ)
            w = gated(wq_w[_rows(half * DM // 2, (half + 1) * DM // 2), :])
            q = mark(jnp.dot(_unpack(x_s[r, half * DM // 2:(half + 1) * DM // 2]), w,
                             preferred_element_type=F32))
            if half == 0:
                st["q", i] = q
            else:
                q_s[i * BQ:(i + 1) * BQ, :] = ((st["q", i] + q) * (HD ** -0.5 * LOG2E)).astype(BF16)

        def kvp(i, which):
            r = _rows(i * BQ, (i + 1) * BQ)
            w = gated(wkv_w[which])
            y = mark(jnp.dot(_unpack(c_s[r, :]), w, preferred_element_type=F32))
            (k_s, v_s)[which][i * BQ:(i + 1) * BQ, :] = y.astype(BF16)

        def Q(*js):
            return [functools.partial(qp, j, half) for j in js for half in range(2)]

        def KV(*js):
            return [functools.partial(kvp, j, w) for j in js for w in range(2)] if project_next else []

        def arrive(*copies):
            def wait():
                @pl.when(h == 0)
                def _():
                    for cp in copies:
                        cp.wait()
            return [wait]

        def X(*blocks):
            return [row_copy(x_hbm, x_s, xsem, i) for i in blocks]

        if prologue:
            units = arrive(w_copy(1, 0), w_copy(2, 0)) + [lambda: unpack_kv(h)]
            for blocks in ((0, 1), (2, 3, 4), (5, 6, 7)):
                units += arrive(*[row_copy(c_hbm, c_s, csem, i) for i in blocks]) + KV(*blocks)
            units += arrive(w_copy(0, 0), *X(7, 6)) + [lambda: unpack_q(h)] + Q(NQ - 1)
            for u in units:
                u()
            return

        rows = S // H
        hr = H - 1 - h
        xr = pl.ds(pl.multiple_of(hr * (rows // 2), rows // 2), rows // 2)
        gw = gw_ref[...].astype(F32).reshape(1, DM)
        gl = functools.reduce(jnp.add, [
            _unpack(x_s[xr, n * L:(n + 1) * L]).astype(F32) * gw[:, n * L:(n + 1) * L] for n in range(NG)])
        gl = jnp.sum(gl, axis=-1, keepdims=True)
        g_s[pl.ds(pl.multiple_of(hr * rows, rows), rows), :] = jnp.broadcast_to(
            jax.nn.sigmoid(gl), (rows, L))

        QN = ([lambda: unpack_q(h + 1)] + Q(NQ - 1)) if project_next else []
        UK = [lambda: unpack_kv(h + 1)] if project_next else []
        if project_next:
            fill = {7: UK + Q(6, 5), 6: Q(4, 3), 5: Q(2) + KV(7), 4: Q(1) + KV(6), 3: Q(0) + KV(5),
                    2: KV(4), 1: QN + KV(3), 0: KV(2), -1: KV(1, 0)}
        else:
            fill = {i: Q(i - 1) if i > 0 else [] for i in range(-1, NQ)}

        for i in range(NQ - 1, -2, -1):
            a = [functools.partial(qk, i, g) for g in range(len(groups(i)))] if i >= 0 else []
            b = [functools.partial(pv, i + 1, g) for g in range(len(groups(i + 1)))] if i + 1 < NQ else []
            units = (a + fill[i]) if i == NQ - 1 else _spread(a, fill[i], b)
            if not project_next and i in (6, 4):
                units = arrive(*X(*{6: (5, 4), 4: (3, 2, 1, 0)}[i])) + units
            for u in units:
                u()

    def head_step(h, carry):
        @pl.when((h & 1) == 1)
        def _next_weights():
            pair = (h + 1) >> 1
            for n in range(3):
                w_copy(n, pair).wait()

            @pl.when(pair + 1 < H // 2)
            def _():
                for n in range(3):
                    w_copy(n, pair + 1).start()

        attention(h, _Order(fwd_ref))
        return carry

    def mix_step(g, carry):
        slot = g & 1
        for cp in g_copies(g):
            cp.wait()

        @pl.when(g + 1 < NG)
        def _():
            for cp in g_copies(g + 1):
                cp.start()

        @pl.when(g >= 2)
        def _():
            o_copy(g - 2).wait()

        cols = pl.ds(pl.multiple_of(g * L, L), L)

        order = _Order(fwd_ref)
        st = {}
        fwd = fwd_ref[...]
        inv = inv_ref[...]
        sk = sk_ref[:, cols].astype(F32)
        sd = sd_s[:, cols]
        hq = CB // 2

        def combine(i, term):
            r = slice(i * CB, (i + 1) * CB)
            if ("half", i) in st:
                o_b[slot, r, :] = (b_s[r, :] + term).astype(BF16)
            else:
                st["half", i] = True
                b_s[r, :] = term

        def out_proj(j, part):
            hs = range(part * HP, (part + 1) * HP)
            w = order.weights(wo_b[slot, _rows(hs[0] * HD, (hs[-1] + 1) * HD), :])
            b = order.mark(jnp.dot(wide(ctx_w, _rows(j * CB, (j + 1) * CB), hs), w,
                                   preferred_element_type=F32))
            b = b if part == 0 else st["b", j] + b
            st["b", j] = b
            if hs[-1] == H - 1:
                combine(j, (1.0 - g_s[j * CB:(j + 1) * CB, :]) * b)

        def shift_mul(i):
            taps = [order.tie(jnp.broadcast_to(sk[t:t + 1, :], (8, L)), 1) for t in range(4)]
            taps = [jnp.concatenate([t] * (CB // 8), axis=0) for t in taps]
            acc = kp_s[8 + i * CB:8 + (i + 1) * CB, :] * taps[0]
            for t in range(1, 4):
                acc = acc + kp_s[8 - t + i * CB:8 - t + (i + 1) * CB, :] * taps[t]
            v = _unpack(av_b[slot, _rows(i * CB, (i + 1) * CB), :]).astype(F32)
            kv_s[i * CB:(i + 1) * CB, :] = (acc * v).astype(BF16)

        def x_spectra(i0):
            w = jnp.concatenate([kv_w[_rows(i * CB, (i + 1) * CB), :] for i in range(i0, i0 + 4)], axis=1)
            xf = order.mark(jnp.dot(fwd, order.weights(w), preferred_element_type=F32))
            for u in range(4):
                xf_s[i0 + u] = xf[:, u * L:(u + 1) * L]

        def h_spectra(m0):
            w = jnp.concatenate([hk_b[slot, :, m * CB:(m + 1) * CB] for m in range(m0, m0 + 4)], axis=0)
            hf4 = order.mark(lax.dot_general(fwd, order.weights(w), NT, preferred_element_type=F32))
            for u in range(4):
                m = m0 + u
                hf = hf4[:, u * L:(u + 1) * L]
                if m == 0:
                    hf_s[m] = hf
                else:
                    prev = st["h"]
                    hf_s[m, 0:hq, :] = hf[0:hq] - prev[2 * hq:3 * hq]
                    hf_s[m, hq:2 * hq, :] = hf[hq:2 * hq] + prev[3 * hq:4 * hq]
                    hf_s[m, 2 * hq:3 * hq, :] = hf[2 * hq:3 * hq] + prev[0:hq]
                    hf_s[m, 3 * hq:4 * hq, :] = hf[3 * hq:4 * hq] - prev[hq:2 * hq]
                st["h"] = hf

        def block_conv(f0, i0, m, frac):
            re = slice(f0, f0 + 8)
            im = slice(CB + f0, CB + f0 + 8)
            if m == 0:
                st["z"] = [None] * TI, [None] * TI
            ar, ai = st["z"]
            gr = order.tie(hf_s[m, re, :], 1, frac)
            gi = order.tie(hf_s[m, im, :], 1, frac)
            for u in range(TI):
                d = i0 + u - m
                if d < 0:
                    continue
                xr = xf_s[d, re, :]
                xi = xf_s[d, im, :]
                pr = gr * xr - gi * xi
                pi = gr * xi + gi * xr
                ar[u] = pr if ar[u] is None else ar[u] + pr
                ai[u] = pi if ai[u] is None else ai[u] + pi
                if d == 0:
                    z_s[i0 + u, re, :] = ar[u]
                    z_s[i0 + u, im, :] = ai[u]

        def finish(i0):
            z = jnp.concatenate([z_s[i0], z_s[i0 + 1]], axis=1).astype(BF16)
            y = order.mark(jnp.dot(inv, z, preferred_element_type=F32))
            for u in range(2):
                i = i0 + u
                r = slice(i * CB, (i + 1) * CB)
                rw = _rows(i * CB, (i + 1) * CB)
                a = _unpack(x_s[rw, cols]).astype(F32) * (
                    y[:, u * L:(u + 1) * L] + _unpack(kv_w[rw, :]).astype(F32) * sd)
                combine(i, g_s[r, :] * a)

        P = functools.partial
        np_ = H // HP
        O = [P(out_proj, j, part) for j in range(NB) for part in range(np_)]
        kp_s[0:8, :] = jnp.zeros((8, L), F32)
        kp_s[8:, :] = _unpack(ak_b[slot]).astype(F32)
        n1, n2, n3 = N1 * np_, N2 * np_, N3 * np_
        units = _spread(O[:n1], [P(h_spectra, m) for m in range(0, NB, 4)],
                        [P(shift_mul, i) for i in range(NB)])
        units += _spread([P(x_spectra, i) for i in range(0, NB, 4)], O[n1:n2])
        conv = [(f0, i0, m) for f0 in range(0, CB, 8) for i0 in range(0, NB, TI) for m in range(i0 + TI)]
        cost = np.array([min(TI, i0 + TI - m) for _, i0, m in conv])
        pos = (np.cumsum(cost) - cost) / cost.sum() * (n3 - n2)
        keyed = [(t + 1e-6, P(block_conv, *c, t % 1.0)) for t, c in zip(pos, conv)]
        keyed += [(n, u) for n, u in enumerate(O[n2:n3])]
        units += [u for _, u in sorted(keyed, key=lambda t: t[0])]
        fin = [P(finish, i) for i in range(0, NB, 2)]
        units += _spread(O[n3:-TAIL], fin) + O[-TAIL:]
        for u in units:
            u()
        o_copy(g).start()
        return carry

    w_copy(1, 0).start()
    w_copy(2, 0).start()
    for i in range(NQ):
        row_copy(c_hbm, c_s, csem, i).start()
    w_copy(0, 0).start()
    for i in reversed(range(NQ)):
        row_copy(x_hbm, x_s, xsem, i).start()
    for n in range(3):
        w_copy(n, 1).start()
    sd_s[...] = sd_ref[...].astype(F32).reshape(1, DM)

    def head_pass(p, carry):
        attention(p, _Order(fwd_ref), prologue=True)
        lax.fori_loop(1, 1 + p * (H - 2), head_step, 0)

        @pl.when(p == 1)
        def _():
            for cp in g_copies(0):
                cp.start()

        attention(p * (H - 1), _Order(fwd_ref), project_next=False)
        return carry

    lax.fori_loop(0, 2, head_pass, 0)
    lax.fori_loop(0, NG, mix_step, 0)
    o_copy(NG - 2).wait()
    o_copy(NG - 1).wait()


@jax.jit
def pallas_gated_mix__ssm_conv_h3__compressed_kv_cla__prompt_kernel(
    A_q: jax.Array,
    A_k: jax.Array,
    A_v: jax.Array,
    A_shift_k: jax.Array,
    A_ssm_k: jax.Array,
    A_ssm_D: jax.Array,
    B_x: jax.Array,
    B_c_kv: jax.Array,
    B_w_q: jax.Array,
    B_w_uk: jax.Array,
    B_w_uv: jax.Array,
    B_w_o: jax.Array,
    gate_w: jax.Array,
):
    del B_x
    hbm = pl.BlockSpec(memory_space=pl.ANY)
    vmem = pl.BlockSpec(memory_space=pltpu.VMEM)
    out = pl.pallas_call(
        _kernel,
        in_specs=[hbm] * 9 + [vmem] * 5,
        out_specs=hbm,
        out_shape=jax.ShapeDtypeStruct((S, DM), BF16),
        scratch_shapes=[
            pltpu.VMEM((S // 2, DM), U32),
            pltpu.VMEM((S // 2, DC), U32),
            pltpu.VMEM((S, HD), BF16),
            pltpu.VMEM((S, HD), BF16),
            pltpu.VMEM((S, HD), BF16),
            pltpu.VMEM((H, S, HD), BF16),
            pltpu.VMEM((S, L), F32),
            pltpu.VMEM((2, DM, HD), U32),
            pltpu.VMEM((2, DC, HD), U32),
            pltpu.VMEM((2, DC, HD), U32),
            pltpu.VMEM((DM, HD), BF16),
            pltpu.VMEM((2, DC, HD), BF16),
            pltpu.VMEM((2, S // 2, L), U32),
            pltpu.VMEM((2, S // 2, L), U32),
            pltpu.VMEM((2, L // 2, S), U32),
            pltpu.VMEM((2, H * HD // 2, L), U32),
            pltpu.VMEM((2, S, L), BF16),
            pltpu.VMEM((1, DM), F32),
            pltpu.VMEM((S + 8, L), F32),
            pltpu.VMEM((NB, 2 * CB, L), F32),
            pltpu.VMEM((NB, 2 * CB, L), F32),
            pltpu.VMEM((NB, 2 * CB, L), F32),
            pltpu.VMEM((S, L), F32),
            pltpu.VMEM((S, L), BF16),
            pltpu.SemaphoreType.DMA((NQ,)),
            pltpu.SemaphoreType.DMA((NQ,)),
            pltpu.SemaphoreType.DMA((3, 2)),
            pltpu.SemaphoreType.DMA((4, 2)),
            pltpu.SemaphoreType.DMA((2,)),
        ],
        compiler_params=pltpu.CompilerParams(vmem_limit_bytes=110 * 1024 * 1024),
    )(
        A_q.reshape(S, DM),
        B_c_kv.reshape(S, DC),
        B_w_q,
        B_w_uk,
        B_w_uv,
        A_k.reshape(S, DM),
        A_v.reshape(S, DM),
        A_ssm_k,
        B_w_o.reshape(H * HD, DM),
        gate_w,
        A_shift_k.T,
        A_ssm_D,
        _FWD_NP,
        _INV_NP,
    )
    return out.reshape(1, S, DM)
```

```python
import functools

import numpy as np

import jax
import jax.numpy as jnp
from jax import lax
import jax.experimental.pallas as pl
import jax.experimental.pallas.tpu as pltpu

S = 2048
DM = 1024
H = 32
HD = 128
DC = 512
L = 128
CB = 128
NB = S // CB
NG = DM // L
BQ = 256
NQ = S // BQ
LAG = 2
HP = 4
TI = 8
TAIL = 4
N1 = 16
N2 = 24
N3 = 104
GS = 4

LOG2E = 1.4426950408889634
NN = (((1,), (0,)), ((), ()))
NT = (((1,), (1,)), ((), ()))
F32 = jnp.float32
BF16 = jnp.bfloat16
U32 = jnp.uint32


def _dft_matrices():
    n = 2 * CB
    f = np.arange(0, CB, 2)
    j = np.arange(CB)
    ang = 2.0 * np.pi * np.outer(np.concatenate([f, CB - 1 - f]) + 0.5, j) / n
    fwd = np.concatenate([np.cos(ang), -np.sin(ang)], axis=0)
    ang = ang[:CB // 2].T[np.concatenate([j[0::2], j[1::2]])]
    inv = np.concatenate([np.cos(ang), -np.sin(ang)], axis=1) * (2.0 / n)
    return fwd.astype(np.float32).astype(BF16), inv.astype(np.float32).astype(BF16)


_FWD_NP, _INV_NP = _dft_matrices()


def _unpack(w):
    return pltpu.bitcast(w, BF16)


def _rows(r0, r1):
    return slice(r0 // 2, r1 // 2)


def _head_weight(w32, h):
    sh = (16 - 16 * (h & 1)).astype(U32)
    return pltpu.bitcast((w32 << sh) & U32(0xFFFF0000), F32)


class _Order:
    def __init__(self, dft_ref):
        self.never = dft_ref[0:16, :].astype(F32)[0:1, :] > 2.0
        self.marks = []

    def mark(self, y):
        self.marks.append(y)
        return y

    def tie(self, a, lag, frac=0.0):
        if len(self.marks) < lag:
            return a
        y = self.marks[-lag]
        r = int(frac * (y.shape[0] // 8)) * 8
        dep = y[r:r + 8, :L]
        if a.dtype == U32:
            dep = pltpu.bitcast(dep, U32)
        n = a.shape[0]
        return jnp.where(self.never, jnp.concatenate([dep] * (n // 8), axis=0), a)

    def trickle(self, a, lag, r0):
        return jnp.where(self.never, self.marks[-lag][r0:r0 + L, :L], a)

    def weights(self, w32, lag=2):
        rows = []
        for r in range(0, w32.shape[0], L // 2):
            head = [self.tie(w32[r:r + 8, c:c + L], lag) for c in range(0, w32.shape[1], L)]
            rows += [jnp.concatenate(head, axis=1), w32[r + 8:r + L // 2]]
        return _unpack(jnp.concatenate(rows, axis=0))


def _spread(*seqs):
    keyed = [((n + 0.5) / len(q) + 1e-3 * k, u) for k, q in enumerate(seqs) for n, u in enumerate(q)]
    return [u for _, u in sorted(keyed, key=lambda t: t[0])]


def _kernel(x_hbm, c_hbm, wq_hbm, wuk_hbm, wuv_hbm, ak_hbm, av_hbm, hk_hbm, wo_hbm,
            gw_ref, sk_ref, sd_ref, fwd_ref, inv_ref,
            o_hbm,
            x_s, c_s, q_s, k_s, v_s, ctx_s, g_s, wq_b, wuk_b, wuv_b, wq_s, wkv_s,
            ak_b, av_b, hk_b, wo_b, o_b, sd_s, kp_s, xf_s, hf_s, z_s, y_s, b_s, kv_s,
            xsem, csem, wsem, gsem, osem):

    q_w, k_w, v_w, ctx_w, wq_w, wkv_w, kv_w = (
        r.bitcast(U32) for r in (q_s, k_s, v_s, ctx_s, wq_s, wkv_s, kv_s))

    def row_copy(src, dst, sem, i):
        r = pl.ds(i * BQ // 2, BQ // 2)
        return pltpu.make_async_copy(src.bitcast(U32).at[r, :], dst.at[r, :], sem.at[i])

    def w_copy(n, pair):
        src, dst = ((wq_hbm, wq_b), (wuk_hbm, wuk_b), (wuv_hbm, wuv_b))[n]
        slot = pair & 1
        return pltpu.make_async_copy(src.bitcast(U32).at[:, pair, :], dst.at[slot], wsem.at[n, slot])

    def g_copies(g):
        slot = g & 1
        cols = pl.ds(pl.multiple_of(g * L, L), L)
        chans = pl.ds(pl.multiple_of(g * (L // 2), L // 2), L // 2)
        srcs = (ak_hbm.bitcast(U32).at[:, cols], av_hbm.bitcast(U32).at[:, cols],
                hk_hbm.bitcast(U32).at[chans, :], wo_hbm.bitcast(U32).at[:, cols])
        return [pltpu.make_async_copy(src, dst.at[slot], gsem.at[n, slot])
                for n, (src, dst) in enumerate(zip(srcs, (ak_b, av_b, hk_b, wo_b)))]

    def o_copy(g):
        slot = g & 1
        return pltpu.make_async_copy(
            o_b.at[slot], o_hbm.at[:, pl.ds(pl.multiple_of(g * L, L), L)], osem.at[slot])

    def unpack_q(h):
        wq_s[...] = _head_weight(wq_b[(h >> 1) & 1], h).astype(BF16)

    def unpack_kv(h):
        slot = (h >> 1) & 1
        wkv_s[0] = _head_weight(wuk_b[slot], h).astype(BF16)
        wkv_s[1] = _head_weight(wuv_b[slot], h).astype(BF16)

    def wide(ref, rows, tiles):
        return jnp.concatenate([_unpack(ref[n, rows, :]) for n in tiles], axis=1)

    def attention(h, order, prologue=False, project_next=True):
        st = {}
        hb = BQ // 2
        row = lax.broadcasted_iota(jnp.int32, (hb, hb), 0)
        col = lax.broadcasted_iota(jnp.int32, (hb, hb), 1)
        tri = col <= row
        neg = -1e9 * LOG2E
        never, gated, mark = order.never, order.weights, order.mark

        def groups(i):
            nt = 2 * i + 1
            return [(j, min(j + GS, nt)) for j in range(0, nt, GS)]

        def qk(i, g):
            r0, r1, r2 = i * BQ, i * BQ + hb, (i + 1) * BQ
            j0, j1 = groups(i)[g]
            d = st.setdefault(i, dict(t={}, b={}, acc=[None, None], o=None, n=0))
            kk = gated(k_w[_rows(j0 * hb, j1 * hb), :])
            s = lax.dot_general(_unpack(q_w[_rows(r0, r2), :]), kk, NT, preferred_element_type=F32)
            for j in range(j1 - j0):
                d["t"][j0 + j] = s[:hb, j * hb:(j + 1) * hb]
                d["b"][j0 + j] = s[hb:, j * hb:(j + 1) * hb]
            if g == len(groups(i)) - 1:
                kl = gated(k_w[_rows(r1, r2), :])
                sl = lax.dot_general(_unpack(q_w[_rows(r1, r2), :]), kl, NT, preferred_element_type=F32)
                d["t"][j1 - 1] = jnp.where(tri, d["t"][j1 - 1], neg)
                d["b"][j1] = jnp.where(tri, sl, neg)
            d["n"] += 1
            if d["n"] == len(groups(i)):
                d["t"], d["b"] = ([t[j] for j in sorted(t)] for t in (d["t"], d["b"]))
                d["m"] = [jnp.max(functools.reduce(jnp.maximum, tiles), axis=-1, keepdims=True)
                          for tiles in (d["t"], d["b"])]
            if j1 - j0 >= 3:
                mark(s)

        def pv(i, g):
            r0, r1, r2 = i * BQ, i * BQ + hb, (i + 1) * BQ
            j0, j1 = groups(i)[g]
            d = st[i]
            last = g == len(groups(i)) - 1
            ps = []
            for half, tiles in enumerate((d["t"], d["b"])):
                tl = tiles[j0:] if last else tiles[j0:j1]
                acc = d["acc"][half]
                m = d["m"][half]
                if g > 0:
                    m = order.trickle(m, LAG, half * hb)
                out = []
                for j, t in enumerate(tl):
                    p = jnp.exp2(t - m)
                    acc = p if acc is None else acc + p
                    if j == len(tl) - 1:
                        if acc is not p:
                            p = jnp.where(never, acc, p)
                        if last and (i + 1) in st:
                            p = jnp.where(never, st[i + 1]["out"][half], p)
                    out.append(p)
                d["acc"][half] = acc
                ps.append(out)
            lhs = jnp.concatenate([jnp.concatenate(ps[0], axis=1),
                                   jnp.concatenate(ps[1][:j1 - j0], axis=1)], axis=0).astype(BF16)
            vv = gated(v_w[_rows(j0 * hb, j1 * hb), :])
            o = jnp.dot(lhs, vv, preferred_element_type=F32)
            d["o"] = o if d["o"] is None else d["o"] + o
            if last:
                vl = gated(v_w[_rows(r1, r2), :])
                ol = jnp.dot(ps[1][-1].astype(BF16), vl, preferred_element_type=F32)
                lt, lb = [jnp.sum(a, axis=-1, keepdims=True) for a in d["acc"]]
                d["out"] = (d["o"][:hb] / lt, (d["o"][hb:] + ol) / lb)
                ctx_s[h, r0:r1, :] = d["out"][0].astype(BF16)
                ctx_s[h, r1:r2, :] = d["out"][1].astype(BF16)
            if j1 - j0 >= 3:
                mark(o)

        def qp(i, half):
            r = _rows(i * BQ, (i + 1) * BQ)
            w = gated(wq_w[_rows(half * DM // 2, (half + 1) * DM // 2), :])
            q = mark(jnp.dot(_unpack(x_s[r, half * DM // 2:(half + 1) * DM // 2]), w,
                             preferred_element_type=F32))
            if half == 0:
                st["q", i] = q
            else:
                q_s[i * BQ:(i + 1) * BQ, :] = ((st["q", i] + q) * (HD ** -0.5 * LOG2E)).astype(BF16)

        def kvp(i, which):
            r = _rows(i * BQ, (i + 1) * BQ)
            w = gated(wkv_w[which])
            y = mark(jnp.dot(_unpack(c_s[r, :]), w, preferred_element_type=F32))
            (k_s, v_s)[which][i * BQ:(i + 1) * BQ, :] = y.astype(BF16)

        def Q(*js):
            return [functools.partial(qp, j, half) for j in js for half in range(2)]

        def KV(*js):
            return [functools.partial(kvp, j, w) for j in js for w in range(2)] if project_next else []

        def arrive(*copies):
            def wait():
                @pl.when(h == 0)
                def _():
                    for cp in copies:
                        cp.wait()
            return [wait]

        def X(*blocks):
            return [row_copy(x_hbm, x_s, xsem, i) for i in blocks]

        if prologue:
            units = arrive(w_copy(1, 0), w_copy(2, 0)) + [lambda: unpack_kv(h)]
            for blocks in ((0, 1), (2, 3, 4), (5, 6, 7)):
                units += arrive(*[row_copy(c_hbm, c_s, csem, i) for i in blocks]) + KV(*blocks)
            units += arrive(w_copy(0, 0), *X(7, 6)) + [lambda: unpack_q(h)] + Q(NQ - 1)
            for u in units:
                u()
            return

        rows = S // H
        hr = H - 1 - h
        xr = pl.ds(pl.multiple_of(hr * (rows // 2), rows // 2), rows // 2)
        gw = gw_ref[...].astype(F32).reshape(1, DM)
        gl = functools.reduce(jnp.add, [
            _unpack(x_s[xr, n * L:(n + 1) * L]).astype(F32) * gw[:, n * L:(n + 1) * L] for n in range(NG)])
        gl = jnp.sum(gl, axis=-1, keepdims=True)
        g_s[pl.ds(pl.multiple_of(hr * rows, rows), rows), :] = jnp.broadcast_to(
            jax.nn.sigmoid(gl), (rows, L))

        QN = ([lambda: unpack_q(h + 1)] + Q(NQ - 1)) if project_next else []
        UK = [lambda: unpack_kv(h + 1)] if project_next else []
        if project_next:
            fill = {7: UK + Q(6, 5), 6: Q(4, 3), 5: Q(2) + KV(7), 4: Q(1) + KV(6), 3: Q(0) + KV(5),
                    2: KV(4), 1: QN + KV(3), 0: KV(2), -1: KV(1, 0)}
        else:
            fill = {i: Q(i - 1) if i > 0 else [] for i in range(-1, NQ)}

        for i in range(NQ - 1, -2, -1):
            a = [functools.partial(qk, i, g) for g in range(len(groups(i)))] if i >= 0 else []
            b = [functools.partial(pv, i + 1, g) for g in range(len(groups(i + 1)))] if i + 1 < NQ else []
            units = (a + fill[i]) if i == NQ - 1 else _spread(a, fill[i], b)
            if not project_next and i in (6, 4):
                units = arrive(*X(*{6: (5, 4), 4: (3, 2, 1, 0)}[i])) + units
            for u in units:
                u()

    def head_step(h, carry):
        @pl.when((h & 1) == 1)
        def _next_weights():
            pair = (h + 1) >> 1
            for n in range(3):
                w_copy(n, pair).wait()

            @pl.when(pair + 1 < H // 2)
            def _():
                for n in range(3):
                    w_copy(n, pair + 1).start()

        attention(h, _Order(fwd_ref))
        return carry

    def mix_step(g, carry):
        slot = g & 1
        for cp in g_copies(g):
            cp.wait()

        @pl.when(g + 1 < NG)
        def _():
            for cp in g_copies(g + 1):
                cp.start()

        @pl.when(g >= 2)
        def _():
            o_copy(g - 2).wait()

        cols = pl.ds(pl.multiple_of(g * L, L), L)

        order = _Order(fwd_ref)
        st = {}
        fwd = fwd_ref[...]
        inv = inv_ref[...]
        sk = sk_ref[:, cols].astype(F32)
        sd = sd_s[:, cols]
        hq = CB // 2

        def combine(i, term):
            r = slice(i * CB, (i + 1) * CB)
            if ("half", i) in st:
                o_b[slot, r, :] = (b_s[r, :] + term).astype(BF16)
            else:
                st["half", i] = True
                b_s[r, :] = term

        def out_proj(j, part):
            hs = range(part * HP, (part + 1) * HP)
            w = order.weights(wo_b[slot, _rows(hs[0] * HD, (hs[-1] + 1) * HD), :])
            b = order.mark(jnp.dot(wide(ctx_w, _rows(j * CB, (j + 1) * CB), hs), w,
                                   preferred_element_type=F32))
            b = b if part == 0 else st["b", j] + b
            st["b", j] = b
            if hs[-1] == H - 1:
                combine(j, (1.0 - g_s[j * CB:(j + 1) * CB, :]) * b)

        def shift_mul(i):
            taps = [order.tie(jnp.broadcast_to(sk[t:t + 1, :], (8, L)), 1) for t in range(4)]
            taps = [jnp.concatenate([t] * (CB // 8), axis=0) for t in taps]
            acc = kp_s[8 + i * CB:8 + (i + 1) * CB, :] * taps[0]
            for t in range(1, 4):
                acc = acc + kp_s[8 - t + i * CB:8 - t + (i + 1) * CB, :] * taps[t]
            v = _unpack(av_b[slot, _rows(i * CB, (i + 1) * CB), :]).astype(F32)
            kv_s[i * CB:(i + 1) * CB, :] = (acc * v).astype(BF16)

        def x_spectra(i0):
            w = jnp.concatenate([kv_w[_rows(i * CB, (i + 1) * CB), :] for i in range(i0, i0 + 4)], axis=1)
            xf = order.mark(jnp.dot(fwd, order.weights(w), preferred_element_type=F32))
            for u in range(4):
                xf_s[i0 + u] = xf[:, u * L:(u + 1) * L]

        def h_spectra(m0):
            w = jnp.concatenate([hk_b[slot, :, m * CB:(m + 1) * CB] for m in range(m0, m0 + 4)], axis=0)
            hf4 = order.mark(lax.dot_general(fwd, order.weights(w), NT, preferred_element_type=F32))
            for u in range(4):
                m = m0 + u
                hf = hf4[:, u * L:(u + 1) * L]
                if m == 0:
                    hf_s[m] = hf
                else:
                    prev = st["h"]
                    hf_s[m, 0:hq, :] = hf[0:hq] - prev[2 * hq:3 * hq]
                    hf_s[m, hq:2 * hq, :] = hf[hq:2 * hq] + prev[3 * hq:4 * hq]
                    hf_s[m, 2 * hq:3 * hq, :] = hf[2 * hq:3 * hq] + prev[0:hq]
                    hf_s[m, 3 * hq:4 * hq, :] = hf[3 * hq:4 * hq] - prev[hq:2 * hq]
                st["h"] = hf

        def block_conv(f0, i0, mirror, m, frac):
            q0, q1, q2, q3 = (slice(n * hq + f0, n * hq + f0 + 8) for n in range(4))
            re, im = (q1, q3) if mirror else (q0, q2)
            if m == 0:
                st["z"] = [None] * TI, [None] * TI
            ar, ai = st["z"]
            gr = order.tie(hf_s[m, re, :], 1, frac)
            gi = order.tie(hf_s[m, im, :], 1, frac)
            for u in range(TI):
                i = i0 + u
                if i < m:
                    continue
                xr = xf_s[i - m, re, :]
                xi = xf_s[i - m, im, :]
                pr = gr * xr - gi * xi
                pi = gr * xi + gi * xr
                ar[u] = pr if ar[u] is None else ar[u] + pr
                ai[u] = pi if ai[u] is None else ai[u] + pi
                if i == m and not mirror:
                    z_s[i, q0, :] = ar[u]
                    z_s[i, q1, :] = ai[u]
                elif i == m:
                    zr, zi = z_s[i, q0, :], z_s[i, q1, :]
                    z_s[i, q0, :] = zr + ar[u]
                    z_s[i, q1, :] = zi - ai[u]
                    z_s[i, q2, :] = zr - ar[u]
                    z_s[i, q3, :] = zi + ai[u]

        def inverse(i0, odd):
            z = jnp.concatenate([z_s[i, odd * CB:(odd + 1) * CB, :] for i in range(i0, i0 + 4)], axis=1)
            head = jnp.concatenate([order.tie(z[:8, c:c + L], 2) for c in range(0, 4 * L, L)], axis=1)
            z = jnp.concatenate([head, z[8:]], axis=0).astype(BF16)
            y = order.mark(jnp.dot(inv[odd * hq:(odd + 1) * hq], z, preferred_element_type=F32))
            for u in range(4):
                y_s[pl.ds((i0 + u) * CB + odd, hq, stride=2), :] = y[:, u * L:(u + 1) * L]

        def finish(i):
            r = slice(i * CB, (i + 1) * CB)
            rw = _rows(i * CB, (i + 1) * CB)
            skip = jnp.concatenate([order.tie(jnp.broadcast_to(sd, (8, L)), 1)] * (CB // 8), axis=0)
            a = _unpack(x_s[rw, cols]).astype(F32) * (y_s[r, :] + _unpack(kv_w[rw, :]).astype(F32) * skip)
            combine(i, g_s[r, :] * a)

        P = functools.partial
        np_ = H // HP
        O = [P(out_proj, j, part) for j in range(NB) for part in range(np_)]
        kp_s[0:8, :] = jnp.zeros((8, L), F32)
        kp_s[8:, :] = _unpack(ak_b[slot]).astype(F32)
        n1, n2, n3 = N1, N2, N3
        units = _spread(O[:n1], [P(h_spectra, m) for m in range(0, NB, 4)],
                        [P(shift_mul, i) for i in range(NB)])
        units += _spread([P(x_spectra, i) for i in range(0, NB, 4)], O[n1:n2])
        conv = [(f0, i0, mirror, m) for f0 in range(0, hq, 8) for mirror in range(2)
                for i0 in range(0, NB, TI) for m in range(i0 + TI)]
        cost = np.array([min(TI, i0 + TI - m) for _, i0, _, m in conv])
        pos = (np.cumsum(cost) - cost) / cost.sum() * (n3 - n2)
        keyed = [(t + 1e-6, P(block_conv, *c, t % 1.0)) for t, c in zip(pos, conv)]
        keyed += [(n, u) for n, u in enumerate(O[n2:n3])]
        units += [u for _, u in sorted(keyed, key=lambda t: t[0])]
        fin = [u for i0 in range(0, NB, 4)
               for u in [P(inverse, i0, 0), P(inverse, i0, 1)] + [P(finish, i) for i in range(i0, i0 + 4)]]
        units += _spread(O[n3:-TAIL], fin) + O[-TAIL:]
        for u in units:
            u()
        o_copy(g).start()
        return carry

    w_copy(1, 0).start()
    w_copy(2, 0).start()
    for i in range(NQ):
        row_copy(c_hbm, c_s, csem, i).start()
    w_copy(0, 0).start()
    for i in reversed(range(NQ)):
        row_copy(x_hbm, x_s, xsem, i).start()
    for n in range(3):
        w_copy(n, 1).start()
    sd_s[...] = sd_ref[...].astype(F32).reshape(1, DM)

    def head_pass(p, carry):
        attention(p, _Order(fwd_ref), prologue=True)
        lax.fori_loop(1, 1 + p * (H - 2), head_step, 0)

        @pl.when(p == 1)
        def _():
            for cp in g_copies(0):
                cp.start()

        attention(p * (H - 1), _Order(fwd_ref), project_next=False)
        return carry

    lax.fori_loop(0, 2, head_pass, 0)
    lax.fori_loop(0, NG, mix_step, 0)
    o_copy(NG - 2).wait()
    o_copy(NG - 1).wait()


@jax.jit
def pallas_gated_mix__ssm_conv_h3__compressed_kv_cla__prompt_kernel(
    A_q: jax.Array,
    A_k: jax.Array,
    A_v: jax.Array,
    A_shift_k: jax.Array,
    A_ssm_k: jax.Array,
    A_ssm_D: jax.Array,
    B_x: jax.Array,
    B_c_kv: jax.Array,
    B_w_q: jax.Array,
    B_w_uk: jax.Array,
    B_w_uv: jax.Array,
    B_w_o: jax.Array,
    gate_w: jax.Array,
):
    del B_x
    hbm = pl.BlockSpec(memory_space=pl.ANY)
    vmem = pl.BlockSpec(memory_space=pltpu.VMEM)
    out = pl.pallas_call(
        _kernel,
        in_specs=[hbm] * 9 + [vmem] * 5,
        out_specs=hbm,
        out_shape=jax.ShapeDtypeStruct((S, DM), BF16),
        scratch_shapes=[
            pltpu.VMEM((S // 2, DM), U32),
            pltpu.VMEM((S // 2, DC), U32),
            pltpu.VMEM((S, HD), BF16),
            pltpu.VMEM((S, HD), BF16),
            pltpu.VMEM((S, HD), BF16),
            pltpu.VMEM((H, S, HD), BF16),
            pltpu.VMEM((S, L), F32),
            pltpu.VMEM((2, DM, HD), U32),
            pltpu.VMEM((2, DC, HD), U32),
            pltpu.VMEM((2, DC, HD), U32),
            pltpu.VMEM((DM, HD), BF16),
            pltpu.VMEM((2, DC, HD), BF16),
            pltpu.VMEM((2, S // 2, L), U32),
            pltpu.VMEM((2, S // 2, L), U32),
            pltpu.VMEM((2, L // 2, S), U32),
            pltpu.VMEM((2, H * HD // 2, L), U32),
            pltpu.VMEM((2, S, L), BF16),
            pltpu.VMEM((1, DM), F32),
            pltpu.VMEM((S + 8, L), F32),
            pltpu.VMEM((NB, 2 * CB, L), F32),
            pltpu.VMEM((NB, 2 * CB, L), F32),
            pltpu.VMEM((NB, 2 * CB, L), F32),
            pltpu.VMEM((S, L), F32),
            pltpu.VMEM((S, L), F32),
            pltpu.VMEM((S, L), BF16),
            pltpu.SemaphoreType.DMA((NQ,)),
            pltpu.SemaphoreType.DMA((NQ,)),
            pltpu.SemaphoreType.DMA((3, 2)),
            pltpu.SemaphoreType.DMA((4, 2)),
            pltpu.SemaphoreType.DMA((2,)),
        ],
        compiler_params=pltpu.CompilerParams(vmem_limit_bytes=110 * 1024 * 1024),
    )(
        A_q.reshape(S, DM),
        B_c_kv.reshape(S, DC),
        B_w_q,
        B_w_uk,
        B_w_uv,
        A_k.reshape(S, DM),
        A_v.reshape(S, DM),
        A_ssm_k,
        B_w_o.reshape(H * HD, DM),
        gate_w,
        A_shift_k.T,
        A_ssm_D,
        _FWD_NP,
        _INV_NP,
    )
    return out.reshape(1, S, DM)
```

```python
import functools

import numpy as np

import jax
import jax.numpy as jnp
from jax import lax
import jax.experimental.pallas as pl
import jax.experimental.pallas.tpu as pltpu

S = 2048
DM = 1024
H = 32
HD = 128
DC = 512
L = 128
CB = 128
NB = S // CB
NG = DM // L
BQ = 256
NQ = S // BQ
KS = 4
GS = 4
HP = 4
TI = 8
N1, N2, N3, TAIL = 16, 24, 104, 4

LOG2E = 1.4426950408889634
NN = (((1,), (0,)), ((), ()))
NT = (((1,), (1,)), ((), ()))
F32 = jnp.float32
BF16 = jnp.bfloat16
U32 = jnp.uint32


def _dft_matrices():
    n = 2 * CB
    f = np.arange(0, CB, 2)
    j = np.arange(CB)
    ang = 2.0 * np.pi * np.outer(np.concatenate([f, CB - 1 - f]) + 0.5, j) / n
    fwd = np.concatenate([np.cos(ang), -np.sin(ang)], axis=0)
    ang = ang[:CB // 2].T[np.concatenate([j[0::2], j[1::2]])]
    inv = np.concatenate([np.cos(ang), -np.sin(ang)], axis=1) * (2.0 / n)
    return fwd.astype(np.float32).astype(BF16), inv.astype(np.float32).astype(BF16)


_FWD_NP, _INV_NP = _dft_matrices()


def _unpack(w):
    return pltpu.bitcast(w, BF16)


def _rows(r0, r1):
    return slice(r0 // 2, r1 // 2)


def _head_weight(w32, h):
    sh = (16 - 16 * (h & 1)).astype(U32)
    return pltpu.bitcast((w32 << sh) & U32(0xFFFF0000), F32)


class _Order:
    def __init__(self, dft_ref):
        self.never = dft_ref[0:16, :].astype(F32)[0:1, :] > 2.0
        self.marks = []

    def mark(self, y):
        self.marks.append(y)
        return y

    def tie(self, a, lag, frac=0.0):
        if len(self.marks) < lag:
            return a
        y = self.marks[-lag]
        r = int(frac * (y.shape[0] // 8)) * 8
        dep = y[r:r + 8, :L]
        if a.dtype == U32:
            dep = pltpu.bitcast(dep, U32)
        n = a.shape[0]
        return jnp.where(self.never, jnp.concatenate([dep] * (n // 8), axis=0), a)

    def trickle(self, a, lag, r0):
        return jnp.where(self.never, self.marks[-lag][r0:r0 + L, :L], a)

    def weights(self, w32, lag=2):
        rows = []
        for r in range(0, w32.shape[0], L // 2):
            head = [self.tie(w32[r:r + 8, c:c + L], lag) for c in range(0, w32.shape[1], L)]
            rows += [jnp.concatenate(head, axis=1), w32[r + 8:r + L // 2]]
        return _unpack(jnp.concatenate(rows, axis=0))


def _spread(*seqs):
    keyed = [((n + 0.5) / len(q) + 1e-3 * k, u) for k, q in enumerate(seqs) for n, u in enumerate(q)]
    return [u for _, u in sorted(keyed, key=lambda t: t[0])]


def _kernel(x_hbm, c_hbm, wq_hbm, wuk_hbm, wuv_hbm, ak_hbm, av_hbm, hk_hbm, wo_hbm,
            gw_ref, sk_ref, sd_ref, fwd_ref, inv_ref,
            o_hbm,
            x_s, c_s, q_s, k_s, v_s, ctx_s, g_s, wq_b, wuk_b, wuv_b, wq_s, wkv_s,
            ak_b, av_b, hk_b, wo_b, o_b, sd_s, kp_s, xf_s, hf_s, z_s, y_s, b_s, kv_s,
            xsem, csem, wsem, gsem, osem):

    q_w, k_w, v_w, ctx_w, wq_w, wkv_w, kv_w = (
        r.bitcast(U32) for r in (q_s, k_s, v_s, ctx_s, wq_s, wkv_s, kv_s))

    def row_copy(src, dst, sem, i):
        r = pl.ds(i * BQ // 2, BQ // 2)
        return pltpu.make_async_copy(src.bitcast(U32).at[r, :], dst.at[r, :], sem.at[i])

    def w_copy(n, pair):
        src, dst = ((wq_hbm, wq_b), (wuk_hbm, wuk_b), (wuv_hbm, wuv_b))[n]
        slot = pair & 1
        return pltpu.make_async_copy(src.bitcast(U32).at[:, pair, :], dst.at[slot], wsem.at[n, slot])

    def g_copies(g):
        slot = g & 1
        cols = pl.ds(pl.multiple_of(g * L, L), L)
        chans = pl.ds(pl.multiple_of(g * (L // 2), L // 2), L // 2)
        srcs = (ak_hbm.bitcast(U32).at[:, cols], av_hbm.bitcast(U32).at[:, cols],
                hk_hbm.bitcast(U32).at[chans, :], wo_hbm.bitcast(U32).at[:, cols])
        return [pltpu.make_async_copy(src, dst.at[slot], gsem.at[n, slot])
                for n, (src, dst) in enumerate(zip(srcs, (ak_b, av_b, hk_b, wo_b)))]

    def o_copy(g):
        slot = g & 1
        return pltpu.make_async_copy(
            o_b.at[slot], o_hbm.at[:, pl.ds(pl.multiple_of(g * L, L), L)], osem.at[slot])

    def unpack_q(h):
        wq_s[...] = _head_weight(wq_b[(h >> 1) & 1], h).astype(BF16)

    def unpack_kv(h):
        slot = (h >> 1) & 1
        wkv_s[0] = _head_weight(wuk_b[slot], h).astype(BF16)
        wkv_s[1] = _head_weight(wuv_b[slot], h).astype(BF16)

    def wide(ref, rows, tiles):
        return jnp.concatenate([_unpack(ref[n, rows, :]) for n in tiles], axis=1)

    def attention(h, order, prologue=False, project_next=True):
        st = {}
        hb = BQ // 2
        row = lax.broadcasted_iota(jnp.int32, (hb, hb), 0)
        col = lax.broadcasted_iota(jnp.int32, (hb, hb), 1)
        tri = col <= row
        neg = -1e9 * LOG2E
        never, gated, mark = order.never, order.weights, order.mark

        def groups(i):
            nt = 2 * i + 1
            return [(j, min(j + GS, nt)) for j in range(0, nt, GS)]

        def qk(i, g):
            r0, r1, r2 = i * BQ, i * BQ + hb, (i + 1) * BQ
            j0, j1 = groups(i)[g]
            d = st.setdefault(i, dict(t={}, b={}, acc=[None, None], o=None, n=0))
            kk = gated(k_w[_rows(j0 * hb, j1 * hb), :])
            s = lax.dot_general(_unpack(q_w[_rows(r0, r2), :]), kk, NT, preferred_element_type=F32)
            for j in range(j1 - j0):
                d["t"][j0 + j] = s[:hb, j * hb:(j + 1) * hb]
                d["b"][j0 + j] = s[hb:, j * hb:(j + 1) * hb]
            if g == len(groups(i)) - 1:
                kl = gated(k_w[_rows(r1, r2), :])
                sl = lax.dot_general(_unpack(q_w[_rows(r1, r2), :]), kl, NT, preferred_element_type=F32)
                d["t"][j1 - 1] = jnp.where(tri, d["t"][j1 - 1], neg)
                d["b"][j1] = jnp.where(tri, sl, neg)
            d["n"] += 1
            if d["n"] == len(groups(i)):
                d["t"], d["b"] = ([t[j] for j in sorted(t)] for t in (d["t"], d["b"]))
                d["m"] = [jnp.max(functools.reduce(jnp.maximum, tiles), axis=-1, keepdims=True)
                          for tiles in (d["t"], d["b"])]
            if j1 - j0 >= 3:
                mark(s)

        def pv(i, g):
            r0, r1, r2 = i * BQ, i * BQ + hb, (i + 1) * BQ
            j0, j1 = groups(i)[g]
            d = st[i]
            last = g == len(groups(i)) - 1
            ps = []
            for half, tiles in enumerate((d["t"], d["b"])):
                tl = tiles[j0:] if last else tiles[j0:j1]
                acc = d["acc"][half]
                m = d["m"][half]
                if g > 0:
                    m = order.trickle(m, 2, half * hb)
                out = []
                for j, t in enumerate(tl):
                    p = jnp.exp2(t - m)
                    acc = p if acc is None else acc + p
                    if j == len(tl) - 1:
                        if acc is not p:
                            p = jnp.where(never, acc, p)
                        if last and (i + 1) in st:
                            p = jnp.where(never, st[i + 1]["out"][half], p)
                    out.append(p)
                d["acc"][half] = acc
                ps.append(out)
            lhs = jnp.concatenate([jnp.concatenate(ps[0], axis=1),
                                   jnp.concatenate(ps[1][:j1 - j0], axis=1)], axis=0).astype(BF16)
            vv = gated(v_w[_rows(j0 * hb, j1 * hb), :])
            o = jnp.dot(lhs, vv, preferred_element_type=F32)
            d["o"] = o if d["o"] is None else d["o"] + o
            if last:
                vl = gated(v_w[_rows(r1, r2), :])
                ol = jnp.dot(ps[1][-1].astype(BF16), vl, preferred_element_type=F32)
                lt, lb = [jnp.sum(a, axis=-1, keepdims=True) for a in d["acc"]]
                d["out"] = (d["o"][:hb] / lt, (d["o"][hb:] + ol) / lb)
                ctx_s[h, r0:r1, :] = d["out"][0].astype(BF16)
                ctx_s[h, r1:r2, :] = d["out"][1].astype(BF16)
            if j1 - j0 >= 3:
                mark(o)

        def qp(i, half):
            r = _rows(i * BQ, (i + 1) * BQ)
            w = gated(wq_w[_rows(half * DM // 2, (half + 1) * DM // 2), :])
            q = mark(jnp.dot(_unpack(x_s[r, half * DM // 2:(half + 1) * DM // 2]), w,
                             preferred_element_type=F32))
            if half == 0:
                st["q", i] = q
            else:
                q_s[i * BQ:(i + 1) * BQ, :] = ((st["q", i] + q) * (HD ** -0.5 * LOG2E)).astype(BF16)

        def kvp(i, which):
            r = _rows(i * BQ, (i + 1) * BQ)
            w = gated(wkv_w[which])
            y = mark(jnp.dot(_unpack(c_s[r, :]), w, preferred_element_type=F32))
            (k_s, v_s)[which][i * BQ:(i + 1) * BQ, :] = y.astype(BF16)

        def Q(*js):
            return [functools.partial(qp, j, half) for j in js for half in range(2)]

        def KV(*js):
            return [functools.partial(kvp, j, w) for j in js for w in range(2)] if project_next else []

        def arrive(*copies):
            def wait():
                @pl.when(h == 0)
                def _():
                    for cp in copies:
                        cp.wait()
            return [wait]

        def X(*blocks):
            return [row_copy(x_hbm, x_s, xsem, i) for i in blocks]

        if prologue:
            units = arrive(w_copy(1, 0), w_copy(2, 0)) + [lambda: unpack_kv(h)]
            for blocks in ((0, 1), (2, 3, 4), (5, 6, 7)):
                units += arrive(*[row_copy(c_hbm, c_s, csem, i) for i in blocks]) + KV(*blocks)
            units += arrive(w_copy(0, 0), *X(7, 6)) + [lambda: unpack_q(h)] + Q(NQ - 1)
            for u in units:
                u()
            return

        rows = S // H
        hr = H - 1 - h
        xr = pl.ds(pl.multiple_of(hr * (rows // 2), rows // 2), rows // 2)
        gw = gw_ref[...].astype(F32).reshape(1, DM)
        gl = functools.reduce(jnp.add, [
            _unpack(x_s[xr, n * L:(n + 1) * L]).astype(F32) * gw[:, n * L:(n + 1) * L] for n in range(NG)])
        gl = jnp.sum(gl, axis=-1, keepdims=True)
        g_s[pl.ds(pl.multiple_of(hr * rows, rows), rows), :] = jnp.broadcast_to(
            jax.nn.sigmoid(gl), (rows, L))

        QN = ([lambda: unpack_q(h + 1)] + Q(NQ - 1)) if project_next else []
        UK = [lambda: unpack_kv(h + 1)] if project_next else []
        if project_next:
            fill = {7: Q(6) + UK + Q(5), 6: Q(4, 3), 5: Q(2) + KV(7), 4: Q(1) + KV(6), 3: Q(0) + KV(5),
                    2: KV(4), 1: QN + KV(3), 0: KV(2), -1: KV(1, 0)}
        else:
            fill = {i: Q(i - 1) if i > 0 else [] for i in range(-1, NQ)}

        for i in range(NQ - 1, -2, -1):
            a = [functools.partial(qk, i, g) for g in range(len(groups(i)))] if i >= 0 else []
            b = [functools.partial(pv, i + 1, g) for g in range(len(groups(i + 1)))] if i + 1 < NQ else []
            units = (fill[i][:1] + a + fill[i][1:]) if i == NQ - 1 else _spread(a, fill[i], b)
            if not project_next and i in (6, 4):
                units = arrive(*X(*{6: (5, 4), 4: (3, 2, 1, 0)}[i])) + units
            for u in units:
                u()

    def head_step(h, carry):
        @pl.when((h & 1) == 1)
        def _next_weights():
            pair = (h + 1) >> 1
            for n in range(3):
                w_copy(n, pair).wait()

            @pl.when(pair + 1 < H // 2)
            def _():
                for n in range(3):
                    w_copy(n, pair + 1).start()

        attention(h, _Order(fwd_ref))
        return carry

    def mix_step(g, carry):
        slot = g & 1
        for cp in g_copies(g):
            cp.wait()

        @pl.when(g + 1 < NG)
        def _():
            for cp in g_copies(g + 1):
                cp.start()

        @pl.when(g >= 2)
        def _():
            o_copy(g - 2).wait()

        cols = pl.ds(pl.multiple_of(g * L, L), L)

        order = _Order(fwd_ref)
        st = {}
        fwd = fwd_ref[...]
        inv = inv_ref[...]
        sk = sk_ref[:, cols].astype(F32)
        sd = sd_s[:, cols]
        hq = CB // 2

        def combine(i, term):
            r = slice(i * CB, (i + 1) * CB)
            if ("half", i) in st:
                o_b[slot, r, :] = (b_s[r, :] + term).astype(BF16)
            else:
                st["half", i] = True
                b_s[r, :] = term

        def out_proj(j, part):
            hs = range(part * HP, (part + 1) * HP)
            w = order.weights(wo_b[slot, _rows(hs[0] * HD, (hs[-1] + 1) * HD), :])
            b = order.mark(jnp.dot(wide(ctx_w, _rows(j * CB, (j + 1) * CB), hs), w,
                                   preferred_element_type=F32))
            b = b if part == 0 else st["b", j] + b
            st["b", j] = b
            if hs[-1] == H - 1:
                combine(j, (1.0 - g_s[j * CB:(j + 1) * CB, :]) * b)

        def shift_mul(i):
            taps = [order.tie(jnp.broadcast_to(sk[t:t + 1, :], (8, L)), 1) for t in range(KS)]
            taps = [jnp.concatenate([t] * (CB // 8), axis=0) for t in taps]
            acc = kp_s[8 + i * CB:8 + (i + 1) * CB, :] * taps[0]
            for t in range(1, KS):
                acc = acc + kp_s[8 - t + i * CB:8 - t + (i + 1) * CB, :] * taps[t]
            v = _unpack(av_b[slot, _rows(i * CB, (i + 1) * CB), :]).astype(F32)
            kv_s[i * CB:(i + 1) * CB, :] = (acc * v).astype(BF16)

        def x_spectra(i0):
            w = jnp.concatenate([kv_w[_rows(i * CB, (i + 1) * CB), :] for i in range(i0, i0 + 4)], axis=1)
            xf = order.mark(jnp.dot(fwd, order.weights(w), preferred_element_type=F32))
            for u in range(4):
                xf_s[i0 + u] = xf[:, u * L:(u + 1) * L]

        def h_spectra(m0):
            w = jnp.concatenate([hk_b[slot, :, m * CB:(m + 1) * CB] for m in range(m0, m0 + 4)], axis=0)
            hf4 = order.mark(lax.dot_general(fwd, order.weights(w), NT, preferred_element_type=F32))
            for u in range(4):
                m = m0 + u
                hf = hf4[:, u * L:(u + 1) * L]
                if m == 0:
                    hf_s[m] = hf
                else:
                    prev = st["h"]
                    hf_s[m, 0:hq, :] = hf[0:hq] - prev[2 * hq:3 * hq]
                    hf_s[m, hq:2 * hq, :] = hf[hq:2 * hq] + prev[3 * hq:4 * hq]
                    hf_s[m, 2 * hq:3 * hq, :] = hf[2 * hq:3 * hq] + prev[0:hq]
                    hf_s[m, 3 * hq:4 * hq, :] = hf[3 * hq:4 * hq] - prev[hq:2 * hq]
                st["h"] = hf

        def block_conv(f0, i0, mirror, m, frac):
            q0, q1, q2, q3 = (slice(n * hq + f0, n * hq + f0 + 8) for n in range(4))
            re, im = (q1, q3) if mirror else (q0, q2)
            if m == 0:
                st["z"] = [None] * TI, [None] * TI
            ar, ai = st["z"]
            gr = order.tie(hf_s[m, re, :], 1, frac)
            gi = order.tie(hf_s[m, im, :], 1, frac)
            for u in range(TI):
                i = i0 + u
                if i < m:
                    continue
                xr = xf_s[i - m, re, :]
                xi = xf_s[i - m, im, :]
                pr = gr * xr - gi * xi
                pi = gr * xi + gi * xr
                ar[u] = pr if ar[u] is None else ar[u] + pr
                ai[u] = pi if ai[u] is None else ai[u] + pi
                if i == m and not mirror:
                    z_s[i, q0, :] = ar[u]
                    z_s[i, q1, :] = ai[u]
                elif i == m:
                    zr, zi = z_s[i, q0, :], z_s[i, q1, :]
                    z_s[i, q0, :] = zr + ar[u]
                    z_s[i, q1, :] = zi - ai[u]
                    z_s[i, q2, :] = zr - ar[u]
                    z_s[i, q3, :] = zi + ai[u]

        def inverse(i0, odd):
            z = jnp.concatenate([z_s[i, odd * CB:(odd + 1) * CB, :] for i in range(i0, i0 + 4)], axis=1)
            head = jnp.concatenate([order.tie(z[:8, c:c + L], 2) for c in range(0, 4 * L, L)], axis=1)
            z = jnp.concatenate([head, z[8:]], axis=0).astype(BF16)
            y = order.mark(jnp.dot(inv[odd * hq:(odd + 1) * hq], z, preferred_element_type=F32))
            for u in range(4):
                y_s[pl.ds((i0 + u) * CB + odd, hq, stride=2), :] = y[:, u * L:(u + 1) * L]

        def finish(i):
            r = slice(i * CB, (i + 1) * CB)
            rw = _rows(i * CB, (i + 1) * CB)
            skip = jnp.concatenate([order.tie(jnp.broadcast_to(sd, (8, L)), 1)] * (CB // 8), axis=0)
            a = _unpack(x_s[rw, cols]).astype(F32) * (y_s[r, :] + _unpack(kv_w[rw, :]).astype(F32) * skip)
            combine(i, g_s[r, :] * a)

        P = functools.partial
        O = [P(out_proj, j, part) for j in range(NB) for part in range(H // HP)]
        kp_s[0:8, :] = jnp.zeros((8, L), F32)
        kp_s[8:, :] = _unpack(ak_b[slot]).astype(F32)
        units = _spread(O[:N1], [P(h_spectra, m) for m in range(0, NB, 4)],
                        [P(shift_mul, i) for i in range(NB)])
        units += _spread([P(x_spectra, i) for i in range(0, NB, 4)], O[N1:N2])
        conv = [(f0, i0, mirror, m) for f0 in range(0, hq, 8) for mirror in range(2)
                for i0 in range(0, NB, TI) for m in range(i0 + TI)]
        cost = np.array([min(TI, i0 + TI - m) for _, i0, _, m in conv])
        pos = (np.cumsum(cost) - cost) / cost.sum() * (N3 - N2)
        keyed = [(t + 1e-6, P(block_conv, *c, t % 1.0)) for t, c in zip(pos, conv)]
        keyed += [(n, u) for n, u in enumerate(O[N2:N3])]
        units += [u for _, u in sorted(keyed, key=lambda t: t[0])]
        fin = [u for i0 in range(0, NB, 4)
               for u in [P(inverse, i0, 0), P(inverse, i0, 1)] + [P(finish, i) for i in range(i0, i0 + 4)]]
        units += _spread(O[N3:-TAIL], fin) + O[-TAIL:]
        for u in units:
            u()
        o_copy(g).start()
        return carry

    w_copy(1, 0).start()
    w_copy(2, 0).start()
    for i in range(NQ):
        row_copy(c_hbm, c_s, csem, i).start()
    w_copy(0, 0).start()
    for i in reversed(range(NQ)):
        row_copy(x_hbm, x_s, xsem, i).start()
    for n in range(3):
        w_copy(n, 1).start()
    sd_s[...] = sd_ref[...].astype(F32).reshape(1, DM)
    q_s[...] = jnp.zeros(q_s.shape, BF16)

    def head_pass(p, carry):
        attention(p, _Order(fwd_ref), prologue=True)
        lax.fori_loop(1, 1 + p * (H - 2), head_step, 0)

        @pl.when(p == 1)
        def _():
            for cp in g_copies(0):
                cp.start()

        attention(p * (H - 1), _Order(fwd_ref), project_next=False)
        return carry

    lax.fori_loop(0, 2, head_pass, 0)
    lax.fori_loop(0, NG, mix_step, 0)
    o_copy(NG - 2).wait()
    o_copy(NG - 1).wait()


@jax.jit
def pallas_gated_mix__ssm_conv_h3__compressed_kv_cla__prompt_kernel(
    A_q: jax.Array,
    A_k: jax.Array,
    A_v: jax.Array,
    A_shift_k: jax.Array,
    A_ssm_k: jax.Array,
    A_ssm_D: jax.Array,
    B_x: jax.Array,
    B_c_kv: jax.Array,
    B_w_q: jax.Array,
    B_w_uk: jax.Array,
    B_w_uv: jax.Array,
    B_w_o: jax.Array,
    gate_w: jax.Array,
):
    del B_x
    hbm = pl.BlockSpec(memory_space=pl.ANY)
    vmem = pl.BlockSpec(memory_space=pltpu.VMEM)
    out = pl.pallas_call(
        _kernel,
        in_specs=[hbm] * 9 + [vmem] * 5,
        out_specs=hbm,
        out_shape=jax.ShapeDtypeStruct((S, DM), BF16),
        scratch_shapes=[
            pltpu.VMEM((S // 2, DM), U32),
            pltpu.VMEM((S // 2, DC), U32),
            pltpu.VMEM((S, HD), BF16),
            pltpu.VMEM((S, HD), BF16),
            pltpu.VMEM((S, HD), BF16),
            pltpu.VMEM((H, S, HD), BF16),
            pltpu.VMEM((S, L), F32),
            pltpu.VMEM((2, DM, HD), U32),
            pltpu.VMEM((2, DC, HD), U32),
            pltpu.VMEM((2, DC, HD), U32),
            pltpu.VMEM((DM, HD), BF16),
            pltpu.VMEM((2, DC, HD), BF16),
            pltpu.VMEM((2, S // 2, L), U32),
            pltpu.VMEM((2, S // 2, L), U32),
            pltpu.VMEM((2, L // 2, S), U32),
            pltpu.VMEM((2, H * HD // 2, L), U32),
            pltpu.VMEM((2, S, L), BF16),
            pltpu.VMEM((1, DM), F32),
            pltpu.VMEM((S + 8, L), F32),
            pltpu.VMEM((NB, 2 * CB, L), F32),
            pltpu.VMEM((NB, 2 * CB, L), F32),
            pltpu.VMEM((NB, 2 * CB, L), F32),
            pltpu.VMEM((S + 8, L), F32),
            pltpu.VMEM((S, L), F32),
            pltpu.VMEM((S, L), BF16),
            pltpu.SemaphoreType.DMA((NQ,)),
            pltpu.SemaphoreType.DMA((NQ,)),
            pltpu.SemaphoreType.DMA((3, 2)),
            pltpu.SemaphoreType.DMA((4, 2)),
            pltpu.SemaphoreType.DMA((2,)),
        ],
        compiler_params=pltpu.CompilerParams(vmem_limit_bytes=80 * 1024 * 1024),
    )(
        A_q.reshape(S, DM),
        B_c_kv.reshape(S, DC),
        B_w_q,
        B_w_uk,
        B_w_uv,
        A_k.reshape(S, DM),
        A_v.reshape(S, DM),
        A_ssm_k,
        B_w_o.reshape(H * HD, DM),
        gate_w,
        A_shift_k.T,
        A_ssm_D,
        _FWD_NP,
        _INV_NP,
    )
    return out.reshape(1, S, DM)
```
